```python
import os as _os
_os.environ.setdefault("JAX_PLATFORMS", "cpu")
import jax
import jax.numpy as jnp

def _softmax(x, axis=-1):
    return jax.nn.softmax(x, axis=axis)
def _gelu(x):
    return jax.nn.gelu(x, approximate=True)
def _silu(x):
    return jax.nn.silu(x)
def _sigmoid(x):
    return jax.nn.sigmoid(x)
def _layernorm(x, axis=-1, eps=1e-5):
    m = jnp.mean(x, axis=axis, keepdims=True)
    v = jnp.var(x, axis=axis, keepdims=True)
    return (x - m) / jnp.sqrt(v + eps)
def _scatter_add(tgt, idx, src, axis=0):
    return tgt.at[idx].add(src)
def _segment_sum(src, seg, n):
    return jax.ops.segment_sum(src, seg, n)
class _Rng:
    def __init__(self, key):
        self._k = key
    def _next(self):
        self._k, sub = jax.random.split(self._k)
        return sub
    def normal(self, shape):
        return jax.random.normal(self._next(), shape, dtype=jnp.bfloat16)
    def randint(self, lo, hi, shape):
        return jax.random.randint(self._next(), shape, lo, hi, dtype=jnp.int32)
    def uniform(self, shape, lo=0.0, hi=1.0):
        return jax.random.uniform(self._next(), shape, jnp.bfloat16, lo, hi)
    def permutation(self, n):
        return jax.random.permutation(self._next(), n)


kernel_name = 'parallel_sum__grouped_kv_mqa__dense_activation_silu__prompt'

def setup_inputs():
    _rng = _Rng(jax.random.key(int.from_bytes(__import__("os").urandom(4), "little")))
    _w = (lambda a: (lambda t: t.astype(jnp.bfloat16) if jnp.issubdtype(t.dtype, jnp.floating) else t)(jnp.asarray(a)))
    def _A_setup():
        B, S, D, H = 1, 2048, 512, 32
        Dh = D // H
        return {
            "x": _w((lambda *s: _rng.normal(s) * 0.05)(B, S, D)),
            "wq": _w((lambda *s: _rng.normal(s) * 0.05)(D, H * Dh)),
            "wk": _w((lambda *s: _rng.normal(s) * 0.05)(D, Dh)),
            "wv": _w((lambda *s: _rng.normal(s) * 0.05)(D, Dh)),
            "wo": _w((lambda *s: _rng.normal(s) * 0.05)(H * Dh, D)),
        }
    _A_in = _A_setup()

    def _B_setup():
        B, S, D, F = 1, 2048, 512, 1792
        return {
            "x": _w((lambda *s: _rng.normal(s) * 0.05)(B, S, D)),
            "w1": _w((lambda *s: _rng.normal(s) * 0.05)(D, F) * (D ** -0.5)),
            "w2": _w((lambda *s: _rng.normal(s) * 0.05)(F, D) * (F ** -0.5)),
        }
    _B_in = _B_setup()

    return {
        "A_x": _A_in["x"],
        "A_wq": _A_in["wq"],
        "A_wk": _A_in["wk"],
        "A_wv": _A_in["wv"],
        "A_wo": _A_in["wo"],
        "B_x": _B_in["x"],
        "B_w1": _B_in["w1"],
        "B_w2": _B_in["w2"],
    }

def reference(A_x, A_wq, A_wk, A_wv, A_wo, B_x, B_w1, B_w2):
    def _A_ref(x, wq, wk, wv, wo):
        B, S, D = x.shape
        H = 32
        Dh = D // H
        q = (lambda x, *d: x.transpose(*d))((x @ wq).reshape(B, S, H, Dh), 0, 2, 1, 3)
        k = x @ wk
        v = x @ wv
        scores = jnp.einsum("bhqd,bkd->bhqk", q, k) * (Dh ** -0.5)
        p = _softmax(scores, axis=-1)
        o = jnp.einsum("bhqk,bkd->bhqd", p, v)
        return (lambda x, *d: x.transpose(*d))(o, 0, 2, 1, 3).reshape(B, S, H * Dh) @ wo

    def _B_ref(x, w1, w2):
        h = jnp.einsum("bsd,df->bsf", x, w1)
        h = _silu(h)
        out = jnp.einsum("bsf,fd->bsd", h, w2)
        return out

    x = A_x
    xn = _layernorm(x, axis=-1)
    return x + _A_ref(xn, A_wq, A_wk, A_wv, A_wo) + _B_ref(xn, B_w1, B_w2)
```

```python
import functools

import jax
import jax.numpy as jnp
from jax import lax
import jax.experimental.pallas as pl
import jax.experimental.pallas.tpu as pltpu

_H = 32
_TQ = 512
_CK = 128
_HPI = 4
_SKEW = 2
_LN_ROWS = 256
_LOG2E = 1.4426950408889634
_SAFE_LOG2 = 60.0
_V_LO = 2.0 ** -30
_V_HI = 2.0 ** 30

_NT = (((1,), (1,)), ((), ()))
_TN = (((0,), (0,)), ((), ()))


def _kernel(x_ref, wq_ref, wk_ref, wv_ref, wo_ref, w1_ref, w2_ref, o_ref,
            xn_scr, k_scr, vt_scr, wqt_scr, qt_scr, ot_scr, s_scr, stat_scr,
            *, S, D, DH, F):
    f32 = jnp.float32
    bf16 = jnp.bfloat16
    step = pl.program_id(0)
    nck = S // _CK
    G = _CK // 16

    @pl.when(step == 0)
    def _():
        wqt_scr[...] = wq_ref[...].astype(f32).T.astype(bf16)
        wvt = wv_ref[...].astype(f32)
        wvt = jnp.concatenate([wvt, jnp.zeros((D, 128 - DH), f32)], axis=1).T[:DH]
        wvt = wvt.astype(bf16)
        wk = wk_ref[...]

        def ln_body(i, carry):
            kmax, vmax = carry
            r0 = pl.multiple_of(i * _LN_ROWS, _LN_ROWS)
            x = x_ref[pl.ds(r0, _LN_ROWS), :].astype(f32)
            mu = jnp.mean(x, axis=-1, keepdims=True)
            xc = x - mu
            var = jnp.mean(xc * xc, axis=-1, keepdims=True)
            xn = (xc * lax.rsqrt(var + 1e-5)).astype(bf16)
            xn_scr[pl.ds(r0, _LN_ROWS), :] = xn
            k = jnp.dot(xn, wk, preferred_element_type=f32).astype(bf16)
            for c in range(_LN_ROWS // _CK):
                for g in range(G):
                    src = c * _CK + g * 16
                    dst = c * _CK + (G - 1 - g) * 16
                    k_scr[pl.ds(r0 + dst, 16), :] = k[src:src + 16]
            vt = lax.dot_general(wvt, xn, _NT, preferred_element_type=f32).astype(bf16)
            vt_scr[:, pl.ds(r0, _LN_ROWS)] = vt
            kf = k.astype(f32)
            kn2 = jnp.sum(kf * kf, axis=-1, keepdims=True)
            kmax = jnp.maximum(kmax, jnp.max(kn2, axis=0, keepdims=True))
            va = jnp.max(jnp.abs(vt.astype(f32)), axis=-1, keepdims=True)
            vmax = jnp.maximum(vmax, jnp.max(va, axis=0, keepdims=True))
            return kmax, vmax

        kmax, vmax = lax.fori_loop(
            0, S // _LN_ROWS, ln_body,
            (jnp.zeros((1, 1), f32), jnp.zeros((1, 1), f32)))
        stat_scr[0] = kmax[0, 0]
        stat_scr[1] = vmax[0, 0]

    q0 = pl.multiple_of(step * _TQ, _TQ)
    xn = xn_scr[pl.ds(q0, _TQ), :]
    qt = lax.dot_general(wqt_scr[...], xn, _NT, preferred_element_type=f32)
    qt = (qt * (DH ** -0.5 * _LOG2E)).astype(bf16)
    qt_scr[...] = qt
    qf = qt.astype(f32)
    qn2 = jnp.sum((qf * qf).reshape(_H, DH, _TQ), axis=1)
    qmax = jnp.max(jnp.max(qn2, axis=0, keepdims=True), axis=1, keepdims=True)[0, 0]
    vmax = stat_scr[1]
    safe = jnp.logical_and(
        qmax * stat_scr[0] <= _SAFE_LOG2 * _SAFE_LOG2,
        jnp.logical_and(vmax >= _V_LO, vmax <= _V_HI))

    def rev_groups(p):
        return jnp.concatenate(
            [p[g * 16:(g + 1) * 16] for g in reversed(range(G))], axis=0)

    @pl.when(safe)
    def _():
        def heads(hh, carry):
            rs = [pl.multiple_of((hh * _HPI + u) * DH, DH) for u in range(_HPI)]
            qts = [qt_scr[pl.ds(r, DH), :] for r in rs]
            accs = [None] * _HPI
            ls = [None] * _HPI
            tiles = []
            tot = nck * _HPI
            for jj in range(tot + _SKEW):
                if jj < tot:
                    u, c = divmod(jj, nck)
                    s = jnp.dot(k_scr[pl.ds(c * _CK, _CK), :], qts[u],
                                preferred_element_type=f32)
                    p = jnp.exp2(s)
                    ps = p.reshape(_CK // 8, 8, _TQ).sum(axis=0)
                    ls[u] = ps if ls[u] is None else ls[u] + ps
                    tiles.append(rev_groups(p).astype(bf16))
                cc = jj - _SKEW
                if cc >= 0:
                    u, c = divmod(cc, nck)
                    pv = jnp.dot(vt_scr[:, pl.ds(c * _CK, _CK)], tiles[cc],
                                 preferred_element_type=f32)
                    tiles[cc] = None
                    accs[u] = pv if accs[u] is None else accs[u] + pv
                    if c == nck - 1:
                        l = jnp.sum(ls[u], axis=0, keepdims=True)
                        ot_scr[pl.ds(rs[u], DH), :] = (accs[u] / l).astype(bf16)
            return carry

        lax.fori_loop(0, _H // _HPI, heads, 0)

    @pl.when(jnp.logical_not(safe))
    def _():
        def head(h, carry):
            r = pl.multiple_of(h * DH, DH)
            qth = qt_scr[pl.ds(r, DH), :]

            def pass1(c, m):
                c0 = pl.multiple_of(c * _CK, _CK)
                s = jnp.dot(k_scr[pl.ds(c0, _CK), :], qth, preferred_element_type=f32)
                s_scr[pl.ds(c0, _CK), :] = s
                return jnp.maximum(m, s.reshape(_CK // 8, 8, _TQ).max(axis=0))

            m8 = lax.fori_loop(0, nck, pass1, jnp.full((8, _TQ), -jnp.inf, f32))
            m = jnp.max(m8, axis=0, keepdims=True)

            def pass2(c, carry2):
                l8, acc = carry2
                c0 = pl.multiple_of(c * _CK, _CK)
                p = jnp.exp2(s_scr[pl.ds(c0, _CK), :] - m)
                l8 = l8 + p.reshape(_CK // 8, 8, _TQ).sum(axis=0)
                acc = acc + jnp.dot(vt_scr[:, pl.ds(c0, _CK)], rev_groups(p).astype(bf16),
                                    preferred_element_type=f32)
                return l8, acc

            l8, acc = lax.fori_loop(
                0, nck, pass2,
                (jnp.zeros((8, _TQ), f32), jnp.zeros((DH, _TQ), f32)))
            l = jnp.sum(l8, axis=0, keepdims=True)
            ot_scr[pl.ds(r, DH), :] = (acc / l).astype(bf16)
            return carry

        lax.fori_loop(0, _H, head, 0)

    o = ot_scr[...].astype(f32).T.astype(bf16)
    out = x_ref[pl.ds(q0, _TQ), :].astype(f32)
    out = out + jnp.dot(o, wo_ref[...], preferred_element_type=f32)
    h = jnp.dot(xn, w1_ref[...], preferred_element_type=f32)
    h = (h * jax.nn.sigmoid(h)).astype(bf16)
    out = out + jnp.dot(h, w2_ref[...], preferred_element_type=f32)
    o_ref[...] = out.astype(o_ref.dtype)


@jax.jit
def pallas_parallel_sum__grouped_kv_mqa__dense_activation_silu__prompt_kernel(
    A_x: jax.Array,
    A_wq: jax.Array,
    A_wk: jax.Array,
    A_wv: jax.Array,
    A_wo: jax.Array,
    B_x: jax.Array,
    B_w1: jax.Array,
    B_w2: jax.Array,
):
    B, S, D = A_x.shape
    DH = A_wk.shape[1]
    F = B_w1.shape[1]
    assert B == 1 and S % _TQ == 0 and D == _H * DH and DH == 16
    x = A_x.reshape(S, D)

    full = lambda shape: pl.BlockSpec(shape, lambda i: (0,) * len(shape))
    out = pl.pallas_call(
        functools.partial(_kernel, S=S, D=D, DH=DH, F=F),
        grid=(S // _TQ,),
        in_specs=[full((S, D)), full((D, D)), full((D, DH)), full((D, DH)),
                  full((D, D)), full((D, F)), full((F, D))],
        out_specs=pl.BlockSpec((_TQ, D), lambda i: (i, 0)),
        out_shape=jax.ShapeDtypeStruct((S, D), A_x.dtype),
        scratch_shapes=[
            pltpu.VMEM((S, D), jnp.bfloat16),
            pltpu.VMEM((S, DH), jnp.bfloat16),
            pltpu.VMEM((DH, S), jnp.bfloat16),
            pltpu.VMEM((D, D), jnp.bfloat16),
            pltpu.VMEM((D, _TQ), jnp.bfloat16),
            pltpu.VMEM((D, _TQ), jnp.bfloat16),
            pltpu.VMEM((S, _TQ), jnp.float32),
            pltpu.SMEM((2,), jnp.float32),
        ],
        compiler_params=pltpu.CompilerParams(
            dimension_semantics=("arbitrary",),
            vmem_limit_bytes=100 * 1024 * 1024),
    )(x, A_wq, A_wk, A_wv, A_wo, B_w1, B_w2)
    return out.reshape(B, S, D)
```

```python
import functools

import jax
import jax.numpy as jnp
from jax import lax
import jax.experimental.pallas as pl
import jax.experimental.pallas.tpu as pltpu

_H = 32
_TQ = 512
_NL = _TQ // 128
_CK = 128
_GS = 8
_GPC = _CK // _GS
_HPI = 8
_DELTA = 17
_ROT = 4
_RB = 256
_LOG2E = 1.4426950408889634
_SAFE_LOG2 = 58.0
_V_LO = 2.0 ** -30
_V_HI = 2.0 ** 30

_NT = (((1,), (1,)), ((), ()))


def _vpu_runs(c, j):
    a = 12 - _ROT * j
    return [(a, a + 1, a + 2)] if (c + j) % 2 == 0 else [(a, a + 1)]


def _plan(S):
    NG = S // _GS
    gof = lambda j, n: (NG - 1 - n - _ROT * j) % NG
    isv = lambda j, n: any((n % _GPC) in run for run in _vpu_runs(n // _GPC, j))
    vgroups = sorted({gof(j, n) for n in range(NG) for j in range(_NL) if isv(j, n)})
    streams = [[(u, n) for u in range(_HPI) for n in range(NG) if not isv(j, n)]
               for j in range(_NL)]
    assert len({len(s) for s in streams}) == 1
    lastidx = {}
    for j in range(_NL):
        for i, (u, n) in enumerate(streams[j]):
            key = (u, n // _GPC)
            lastidx[key] = max(lastidx.get(key, 0), i)
    return gof, vgroups, streams, lastidx


def _kernel(x_hbm, wq_hbm, wkt_hbm, wvt_hbm, wo_hbm, w1_hbm, w2_hbm, o_ref,
            x_scr, wq_scr, wo_scr, w1_scr, w2_scr, xsem, wsem,
            xn_scr, wt_scr, qt_scr, kt_scr, k_scr, kb_scr, vt_scr, ot_scr, l_scr, s_scr,
            flag_scr, z_scr, *, S, D, DH, F):
    f32 = jnp.float32
    bf16 = jnp.bfloat16
    step = pl.program_id(0)
    nck = S // _CK
    nrb = S // _RB
    gof, vgroups, streams, lastidx = _plan(S)
    kbrow = {g: i * _GS for i, g in enumerate(vgroups)}

    def x_copy(i):
        return pltpu.make_async_copy(
            x_hbm.at[pl.ds(i * _RB, _RB)], x_scr.at[pl.ds(i * _RB, _RB)], xsem.at[i])

    w_copies = [
        pltpu.make_async_copy(wq_hbm, wq_scr, wsem.at[0]),
        pltpu.make_async_copy(wkt_hbm, wt_scr.at[pl.ds(D, DH)], wsem.at[1]),
        pltpu.make_async_copy(wvt_hbm, wt_scr.at[pl.ds(D + DH, DH)], wsem.at[2]),
        pltpu.make_async_copy(wo_hbm, wo_scr, wsem.at[3]),
        pltpu.make_async_copy(w1_hbm, w1_scr, wsem.at[4]),
        pltpu.make_async_copy(w2_hbm, w2_scr, wsem.at[5]),
    ]

    @pl.when(step == 0)
    def _():
        x_copy(0).start()
        for c in w_copies[:3]:
            c.start()
        x_copy(1).start()
        x_copy(2).start()
        for i in range(_HPI * _NL):
            z_scr[i] = 0

        def layernorm(i):
            x = x_scr[pl.ds(i * _RB, _RB), :].astype(f32)
            mu = jnp.mean(x, axis=-1, keepdims=True)
            xc = x - mu
            var = jnp.mean(xc * xc, axis=-1, keepdims=True)
            xn_scr[pl.ds(i * _RB, _RB), :] = (xc * lax.rsqrt(var + 1e-5)).astype(bf16)

        hsel = (lax.broadcasted_iota(jnp.int32, (_H, D), 1) // DH
                == lax.broadcasted_iota(jnp.int32, (_H, D), 0)).astype(f32)

        def project(i):
            xn = xn_scr[pl.ds(i * _RB, _RB), :]
            t = lax.dot_general(wt_scr[...], xn, _NT, preferred_element_type=f32)
            for j in range(_RB // 128):
                qt_scr[i * (_RB // 128) + j] = t[:D, j * 128:(j + 1) * 128]
            kt_scr[:, pl.ds(i * _RB, _RB)] = t[D:D + DH] * (DH ** -0.5 * _LOG2E)
            vt_scr[0, :, pl.ds(i * _RB, _RB)] = t[D + DH:]

        def post(i, stats):
            qmax, kmax, vmax = stats
            kt = kt_scr[:, pl.ds(i * _RB, _RB)]
            vt = vt_scr[0, :, pl.ds(i * _RB, _RB)]
            ktp = jnp.concatenate([kt, jnp.zeros((128 - DH, _RB), f32)], axis=0)
            k = ktp.T[:, :DH]
            k_scr[pl.ds(i * _RB, _RB), :] = k
            g0 = i * _RB // _GS
            gs = [g for g in vgroups if g0 <= g < g0 + _RB // _GS]
            ksel = jnp.concatenate(
                [k[(g - g0) * _GS:(g - g0 + 1) * _GS] for g in gs], axis=0)
            nr = len(gs) * _GS
            for d in range(DH):
                kb_scr[pl.ds(kbrow[gs[0]], nr), pl.ds(d * 128, 128)] = (
                    jnp.broadcast_to(ksel[:, d:d + 1], (nr, 128)))
            q = jnp.concatenate(
                [qt_scr[i * (_RB // 128) + j] for j in range(_RB // 128)], axis=1)
            qn2 = jnp.dot(hsel, q * q, preferred_element_type=f32)
            qmax = jnp.maximum(qmax, qn2)
            kmax = jnp.maximum(kmax, jnp.sum(kt * kt, axis=0, keepdims=True))
            vmax = jnp.maximum(vmax, jnp.abs(vt))
            return qmax, kmax, vmax

        x_copy(0).wait()
        for i in range(3, nrb):
            x_copy(i).start()
        layernorm(0)
        for c in w_copies[:3]:
            c.wait()
        x_copy(1).wait()
        x_copy(2).wait()
        wt_scr[pl.ds(0, D), :] = wq_scr[...].astype(f32).T.astype(bf16)
        stats = (jnp.zeros((_H, _RB), f32), jnp.zeros((1, _RB), f32),
                 jnp.zeros((DH, _RB), f32))
        layernorm(1)
        project(0)
        layernorm(2)
        project(1)
        for i in range(2, nrb + 2):
            if i == 2:
                for ii in range(3, nrb):
                    x_copy(ii).wait()
                for c in w_copies[3:]:
                    c.start()
            if i + 1 < nrb:
                layernorm(i + 1)
            if i < nrb:
                project(i)
            stats = post(i - 2, stats)
        vt_all = vt_scr[0]
        for j in range(1, _NL):
            vt_scr[j] = pltpu.roll(vt_all, _ROT * _GS * j, 1)
        qmax, kmax, vmax = [jnp.max(jnp.max(a, axis=0, keepdims=True), axis=1,
                                    keepdims=True)[0, 0] for a in stats]
        safe = jnp.logical_and(
            qmax * kmax <= _SAFE_LOG2 * _SAFE_LOG2,
            jnp.logical_and(vmax >= _V_LO, vmax <= _V_HI))
        flag_scr[0] = safe.astype(jnp.int32)

    safe = flag_scr[0] == 1
    lt0 = step * _NL

    @pl.when(safe)
    def _():
        def heads(hh, carry):
            rs = [pl.multiple_of((hh * _HPI + u) * DH, DH) for u in range(_HPI)]
            zs = [[pl.multiple_of(z_scr[u * _NL + j], 8) for j in range(_NL)]
                  for u in range(_HPI)]
            kbv = [[kb_scr.at[pl.ds(z, kb_scr.shape[0])] for z in zu] for zu in zs]
            ksv = [[k_scr.at[pl.ds(z, k_scr.shape[0])] for z in zu] for zu in zs]
            qts = [[qt_scr[lt0 + j, pl.ds(r, DH), :] for j in range(_NL)] for r in rs]
            accs = [[None] * _NL for _ in range(_HPI)]
            ls = [[None] * _NL for _ in range(_HPI)]
            P = [dict() for _ in range(_NL)]
            pos = [0] * _NL

            def add_l(u, j, p):
                n = p.shape[0] // 8
                ps = p.reshape(n, 8, 128).sum(axis=0) if n > 1 else p
                ls[u][j] = ps if ls[u][j] is None else ls[u][j] + ps

            def qk_seg(j, end):
                st = streams[j]
                end = min(end, len(st))
                if pos[j] >= end:
                    return False
                u = st[pos[j]][0]
                e = pos[j]
                while e < end and st[e][0] == u:
                    e += 1
                items = st[pos[j]:e]
                kk = jnp.concatenate(
                    [ksv[u][j][pl.ds(gof(j, n) * _GS, _GS), :] for (_, n) in items],
                    axis=0)
                p = jnp.exp2(jnp.dot(kk, qts[u][j], preferred_element_type=f32))
                add_l(u, j, p)
                for i, it in enumerate(items):
                    P[j][it] = p[i * _GS:(i + 1) * _GS]
                pos[j] = e
                return True

            def vpu(u, j, ns):
                ch = [None] * len(ns)
                for d in range(DH):
                    qb = qt_scr[lt0 + j, pl.ds(rs[u] + d, 8, stride=0), :]
                    for i, n in enumerate(ns):
                        kd = kbv[u][j][pl.ds(kbrow[gof(j, n)], _GS), pl.ds(d * 128, 128)]
                        tt = kd * qb
                        ch[i] = tt if ch[i] is None else ch[i] + tt
                p = jnp.exp2(jnp.concatenate(ch, axis=0))
                add_l(u, j, p)
                for i, n in enumerate(ns):
                    P[j][(u, n)] = p[i * _GS:(i + 1) * _GS]

            for m in range(nck * _HPI):
                u, c = divmod(m, nck)
                end = lastidx[(u, c)] + 1 + _DELTA
                more, first = True, True
                while more:
                    more = False
                    for j in range(_NL):
                        more |= qk_seg(j, end)
                        if first:
                            for run in _vpu_runs(c, j):
                                vpu(u, j, [c * _GPC + t for t in run])
                    first = False
                for j in range(_NL):
                    vc = vt_scr[j, :, pl.ds((nck - 1 - c) * _CK, _CK)]
                    tile = jnp.concatenate(
                        [P[j].pop((u, n))
                         for n in reversed(range(c * _GPC, (c + 1) * _GPC))], axis=0)
                    pv = jnp.dot(vc, tile, preferred_element_type=f32)
                    accs[u][j] = pv if accs[u][j] is None else pv + accs[u][j]
                    if c == nck - 1:
                        ot_scr[pl.ds(rs[u], DH), pl.ds(j * 128, 128)] = accs[u][j]
                        l_scr[j, pl.ds(pl.multiple_of((hh * _HPI + u) * 8, 8), 8), :] = (
                            ls[u][j])
            return carry

        lax.fori_loop(0, _H // _HPI, heads, 0)

    @pl.when(jnp.logical_not(safe))
    def _():
        def head(h, carry):
            r = pl.multiple_of(h * DH, DH)
            qth = jnp.concatenate(
                [qt_scr[lt0 + j, pl.ds(r, DH), :] for j in range(_NL)], axis=1)

            def pass1(c, m):
                c0 = pl.multiple_of(c * _CK, _CK)
                s = jnp.dot(k_scr[pl.ds(c0, _CK), :], qth, preferred_element_type=f32)
                s_scr[pl.ds(c0, _CK), :] = s
                return jnp.maximum(m, s.reshape(_CK // 8, 8, _TQ).max(axis=0))

            m8 = lax.fori_loop(0, nck, pass1, jnp.full((8, _TQ), -jnp.inf, f32))
            m = jnp.max(m8, axis=0, keepdims=True)

            def pass2(c, carry2):
                l8, acc = carry2
                c0 = pl.multiple_of(c * _CK, _CK)
                p = jnp.exp2(s_scr[pl.ds(c0, _CK), :] - m)
                l8 = l8 + p.reshape(_CK // 8, 8, _TQ).sum(axis=0)
                acc = acc + jnp.dot(vt_scr[0, :, pl.ds(c0, _CK)], p,
                                    preferred_element_type=f32)
                return l8, acc

            l8, acc = lax.fori_loop(
                0, nck, pass2,
                (jnp.zeros((8, _TQ), f32), jnp.zeros((DH, _TQ), f32)))
            ot_scr[pl.ds(r, DH), :] = acc
            for j in range(_NL):
                l_scr[j, pl.ds(pl.multiple_of(h * 8, 8), 8), :] = (
                    l8[:, j * 128:(j + 1) * 128])
            return carry

        lax.fori_loop(0, _H, head, 0)

    @pl.when(step == 0)
    def _():
        for c in w_copies[3:]:
            c.wait()

    q0 = pl.multiple_of(step * _TQ, _TQ)
    xn = xn_scr[pl.ds(q0, _TQ), :]
    h = jnp.dot(xn, w1_scr[...], preferred_element_type=f32)
    h = (h * jax.nn.sigmoid(h)).astype(bf16)
    out = x_scr[pl.ds(q0, _TQ), :].astype(f32)
    out = jnp.dot(h, w2_scr[...], preferred_element_type=f32) + out
    lsum = []
    for j in range(_NL):
        lj = l_scr[j, pl.ds(0, _H, stride=8), :]
        for sub in range(1, 8):
            lj = lj + l_scr[j, pl.ds(sub, _H, stride=8), :]
        lsum.append(lj)
    rl = 1.0 / jnp.concatenate(lsum, axis=1)
    ot = jnp.concatenate(
        [ot_scr[pl.ds(hd * DH, DH), :] * rl[hd:hd + 1] for hd in range(_H)], axis=0)
    o = ot.T.astype(bf16)
    out = jnp.dot(o, wo_scr[...], preferred_element_type=f32) + out
    o_ref[...] = out.astype(o_ref.dtype)


@jax.jit
def pallas_parallel_sum__grouped_kv_mqa__dense_activation_silu__prompt_kernel(
    A_x: jax.Array,
    A_wq: jax.Array,
    A_wk: jax.Array,
    A_wv: jax.Array,
    A_wo: jax.Array,
    B_x: jax.Array,
    B_w1: jax.Array,
    B_w2: jax.Array,
):
    B, S, D = A_x.shape
    DH = A_wk.shape[1]
    F = B_w1.shape[1]
    assert B == 1 and S % _TQ == 0 and D == _H * DH and DH == 16
    x = A_x.reshape(S, D)
    bf16 = jnp.bfloat16
    f32 = jnp.float32
    nv = len(_plan(S)[1]) * _GS

    hbm = pl.BlockSpec(memory_space=pl.ANY)
    out = pl.pallas_call(
        functools.partial(_kernel, S=S, D=D, DH=DH, F=F),
        grid=(S // _TQ,),
        in_specs=[hbm] * 7,
        out_specs=pl.BlockSpec((_TQ, D), lambda i: (i, 0)),
        out_shape=jax.ShapeDtypeStruct((S, D), A_x.dtype),
        scratch_shapes=[
            pltpu.VMEM((S, D), bf16),
            pltpu.VMEM((D, D), bf16),
            pltpu.VMEM((D, D), bf16),
            pltpu.VMEM((D, F), bf16),
            pltpu.VMEM((F, D), bf16),
            pltpu.SemaphoreType.DMA((S // _RB,)),
            pltpu.SemaphoreType.DMA((6,)),
            pltpu.VMEM((S, D), bf16),
            pltpu.VMEM((D + 2 * DH, D), bf16),
            pltpu.VMEM((S // 128, D, 128), f32),
            pltpu.VMEM((DH, S), f32),
            pltpu.VMEM((S, DH), f32),
            pltpu.VMEM((nv, DH * 128), f32),
            pltpu.VMEM((_NL, DH, S), f32),
            pltpu.VMEM((D, _TQ), f32),
            pltpu.VMEM((_NL, _H * 8, 128), f32),
            pltpu.VMEM((S, _TQ), f32),
            pltpu.SMEM((1,), jnp.int32),
            pltpu.SMEM((_HPI * _NL,), jnp.int32),
        ],
        compiler_params=pltpu.CompilerParams(
            dimension_semantics=("arbitrary",),
            vmem_limit_bytes=100 * 1024 * 1024),
    )(x, A_wq, A_wk.T, A_wv.T, A_wo, B_w1, B_w2)
    return out.reshape(B, S, D)
```

```python
import functools

import jax
import jax.numpy as jnp
from jax import lax
import jax.experimental.pallas as pl
import jax.experimental.pallas.tpu as pltpu

_H = 32
_TQ = 512
_NL = _TQ // 128
_CK = 128
_GS = 8
_GPC = _CK // _GS
_HPI = 8
_DELTA = 16
_ROT = 4
_RB = 256
_NZ = 64
_LOG2E = 1.4426950408889634
_SAFE_LOG2 = 58.0
_V_LO = 2.0 ** -30
_V_HI = 2.0 ** 30
_QG = 4
_PRE = (1, 3, 5, 7)
_CPRE = 14
_HEADPV = (6, 12)
_PACE1 = 18.0
_PACES = (8, 10, 11, 8, 8.5, 13, 9, 8, 13, 8, 14, 13, 16)
_ODOT = 25
_QBN = (0, 32, 20, 12, 12, 12, 16, 24)

_NT = (((1,), (1,)), ((), ()))


def _vpu_run(u, c, j):
    a = 12 - _ROT * j
    big = (c + (j in (0, 3))) % 2 == 0 and not (u in _PRE and c == _CPRE + 1)
    return tuple(range(a, a + (3 if big else 2)))


def _plan(S):
    NG = S // _GS
    nck = S // _CK
    gof = lambda j, n: (NG - 1 - n - _ROT * j) % NG
    tiles = [(u, c) for u in range(_HPI) for c in range(nck)
             if not (u in _PRE and c == _CPRE)]
    vg = {gof(j, _CPRE * _GPC + t) for j in range(_NL) for t in range(_GPC)}
    streams = [[] for _ in range(_NL)]
    for (u, c) in tiles:
        for j in range(_NL):
            for t in range(_GPC):
                if t in _vpu_run(u, c, j):
                    vg.add(gof(j, c * _GPC + t))
                else:
                    streams[j].append((u, c * _GPC + t))
    assert len({len(s) for s in streams}) == 1
    lastidx = {}
    for j in range(_NL):
        for i, (u, n) in enumerate(streams[j]):
            key = (u, n // _GPC)
            lastidx[key] = max(lastidx.get(key, 0), i)
    return gof, sorted(vg), tiles, streams, lastidx


def _dense_slots(paces, nunits):
    slots = {}
    unit, gi = 0, 0
    t = 48.0
    while unit < nunits:
        pace = paces[int(t // 512)]
        rem = _GPC - gi
        n = min(2 if (pace > 12 or rem == 4) else 3, rem)
        t += n * pace
        while (int(t // 512), int(t % 512) // 16) in slots:
            t = (t // 16 + 1) * 16
        assert t < 512 * len(paces)
        slots[(int(t // 512), int(t % 512) // 16)] = (unit, gi, n)
        gi += n
        if gi == _GPC:
            unit, gi = unit + 1, 0
    return slots


def _kernel(x_hbm, wq_hbm, wkt_hbm, wvt_hbm, wo_hbm, w1_hbm, w2_hbm, o_ref,
            x_scr, wq_scr, wo_scr, w1_scr, w2_scr, xsem, wsem,
            xn_scr, wt_scr, qt_scr, kt_scr, k_scr, kb_scr, vt_scr, ot_scr, ot2_scr,
            l_scr, p_scr, lp_scr, h_scr, acc_scr, qb_scr, s_scr, flag_scr, z_scr,
            *, S, D, DH, F):
    f32 = jnp.float32
    bf16 = jnp.bfloat16
    u32 = jnp.uint32
    step = pl.program_id(0)
    nck = S // _CK
    nrb = S // _RB
    gof, vgroups, tiles, streams, lastidx = _plan(S)
    kbrow = {g: i * _GS for i, g in enumerate(vgroups)}
    npre = len(_PRE)
    pre_heads = [it * _HPI + u for it in range(_H // _HPI) for u in _PRE]
    pre_g0 = [gof(j, _CPRE * _GPC + _GPC - 1) for j in range(_NL)]

    def x_copy(i):
        return pltpu.make_async_copy(
            x_hbm.at[pl.ds(i * _RB, _RB)], x_scr.at[pl.ds(i * _RB, _RB)], xsem.at[i])

    w_copies = [
        pltpu.make_async_copy(wq_hbm, wq_scr, wsem.at[0]),
        pltpu.make_async_copy(wkt_hbm, wt_scr.at[pl.ds(D, DH)], wsem.at[1]),
        pltpu.make_async_copy(wvt_hbm, wt_scr.at[pl.ds(D + DH, DH)], wsem.at[2]),
        pltpu.make_async_copy(wo_hbm, wo_scr, wsem.at[3]),
        pltpu.make_async_copy(w1_hbm, w1_scr, wsem.at[4]),
        pltpu.make_async_copy(w2_hbm, w2_scr, wsem.at[5]),
    ]

    def build_qb(lt, hd, j, after=None):
        qq = qt_scr[lt + j, pl.ds(hd * DH, DH), :]
        if after is not None:
            zvec = jnp.full((8, 128), z_scr[0], jnp.int32).astype(u32)
            z = pltpu.bitcast(after, u32) & zvec
            qq = pltpu.bitcast(
                pltpu.bitcast(qq, u32) | jnp.concatenate([z, z], axis=0), f32)
        for d in range(DH):
            qb_scr[j, hd * DH + d] = jnp.broadcast_to(qq[d:d + 1], (8, 128))

    @pl.when(step == 0)
    def _():
        x_copy(0).start()
        for c in w_copies[:3]:
            c.start()
        x_copy(1).start()
        x_copy(2).start()
        for i in range(_NZ):
            z_scr[i] = 0

        def layernorm(i):
            x = x_scr[pl.ds(i * _RB, _RB), :].astype(f32)
            mu = jnp.mean(x, axis=-1, keepdims=True)
            xc = x - mu
            var = jnp.mean(xc * xc, axis=-1, keepdims=True)
            xn_scr[pl.ds(i * _RB // 2, _RB // 2), :] = pltpu.bitcast(
                (xc * lax.rsqrt(var + 1e-5)).astype(bf16), u32)

        def project(i):
            xn = pltpu.bitcast(xn_scr[pl.ds(i * _RB // 2, _RB // 2), :], bf16)
            t = lax.dot_general(wt_scr[...], xn, _NT, preferred_element_type=f32)
            for j in range(_RB // 128):
                qt_scr[i * (_RB // 128) + j] = t[:D, j * 128:(j + 1) * 128]
            kt_scr[:, pl.ds(i * _RB, _RB)] = t[D:D + DH] * (DH ** -0.5 * _LOG2E)
            vt_scr[0, :, pl.ds(i * _RB, _RB)] = t[D + DH:]
            units = range(sum(_QBN[:i]), sum(_QBN[:i + 1]))
            for k, un in enumerate(units):
                cj, rr = divmod(k * 2 * (D // 8) // len(units), D // 8)
                build_qb(0, un % _H, un // _H,
                         t[rr * 8:rr * 8 + 8, cj * 128:(cj + 1) * 128])

        def post(i, stats):
            qmax, kmax, vmax = stats
            kt = kt_scr[:, pl.ds(i * _RB, _RB)]
            vt = vt_scr[0, :, pl.ds(i * _RB, _RB)]
            ktp = jnp.concatenate([kt, jnp.zeros((128 - DH, _RB), f32)], axis=0)
            kp = ktp.T
            k_scr[pl.ds(i * _RB, _RB), :] = kp[:, :DH]
            g0 = i * _RB // _GS
            gs = [g for g in vgroups if g0 <= g < g0 + _RB // _GS]
            ksel = jnp.concatenate(
                [kp[(g - g0) * _GS:(g - g0 + 1) * _GS] for g in gs], axis=0)
            nr = len(gs) * _GS
            lane = lax.broadcasted_iota(jnp.int32, (nr, 128), 1)
            for d in range(DH):
                col = jnp.sum(jnp.where(lane == d, ksel, 0.0), axis=1, keepdims=True)
                kb_scr[pl.ds(kbrow[gs[0]], nr), pl.ds(d * 128, 128)] = (
                    jnp.broadcast_to(col, (nr, 128)))
            q = jnp.concatenate(
                [qt_scr[i * (_RB // 128) + j] for j in range(_RB // 128)], axis=1)
            q2 = (q * q).reshape(_H // _QG, _QG, 2, 8, _RB)
            q2 = jnp.max(q2[:, :, 0] + q2[:, :, 1], axis=1)
            qmax = jnp.maximum(qmax, jnp.max(jnp.sum(q2, axis=1, keepdims=True), axis=0))
            kmax = jnp.maximum(kmax, jnp.sum(kt * kt, axis=0, keepdims=True))
            vmax = jnp.maximum(vmax, jnp.abs(vt))
            return qmax, kmax, vmax

        def pre_tile0(lo, hi):
            for i in range(lo, hi):
                for j in range(_NL):
                    kk = k_scr[pl.ds(pre_g0[j] * _GS, _CK), :]
                    qq = qt_scr[j, pl.ds(pre_heads[i] * DH, DH), :]
                    p = jnp.exp2(jnp.dot(kk, qq, preferred_element_type=f32))
                    p_scr[i * _NL + j] = p
                    lp_scr[i * _NL + j] = p.reshape(_GPC, 8, 128).sum(axis=0)

        x_copy(0).wait()
        for i in range(3, nrb):
            x_copy(i).start()
        layernorm(0)
        for c in w_copies[:3]:
            c.wait()
        wt_scr[pl.ds(0, D), :] = wq_scr[...].astype(f32).T.astype(bf16)
        x_copy(1).wait()
        x_copy(2).wait()
        stats = (jnp.zeros((1, _RB), f32), jnp.zeros((1, _RB), f32),
                 jnp.zeros((DH, _RB), f32))
        layernorm(1)
        project(0)
        layernorm(2)
        project(1)
        for i in range(2, nrb + 2):
            if i == 2:
                for ii in range(3, nrb):
                    x_copy(ii).wait()
                for c in w_copies[3:]:
                    c.start()
            if i + 1 < nrb:
                layernorm(i + 1)
            if i < nrb:
                project(i)
            if i == nrb + 1:
                pre_tile0(0, len(pre_heads) // 2)
            stats = post(i - 2, stats)
        pre_tile0(len(pre_heads) // 2, len(pre_heads))
        vt_all = vt_scr[0]
        for j in range(1, _NL):
            vt_scr[j] = pltpu.roll(vt_all, _ROT * _GS * j, 1)
        qmax, kmax, vmax = [jnp.max(jnp.max(a, axis=0, keepdims=True), axis=1,
                                    keepdims=True)[0, 0] for a in stats]
        safe = jnp.logical_and(
            qmax * kmax <= _SAFE_LOG2 * _SAFE_LOG2,
            jnp.logical_and(vmax >= _V_LO, vmax <= _V_HI))
        flag_scr[0] = safe.astype(jnp.int32)

    safe = flag_scr[0] == 1
    lt0 = step * _NL

    @pl.when(safe)
    def _():
        def heads(hh, carry):
            rs = [pl.multiple_of((hh * _HPI + u) * DH, DH) for u in range(_HPI)]
            zs = [[pl.multiple_of(z_scr[u * _NL + j], 8) for j in range(_NL)]
                  for u in range(_HPI)]
            kbv = [[kb_scr.at[pl.ds(z, kb_scr.shape[0])] for z in zu] for zu in zs]
            ksv = [[k_scr.at[pl.ds(z, k_scr.shape[0])] for z in zu] for zu in zs]
            qts = [[qt_scr[lt0 + j, pl.ds(r, DH), :] for j in range(_NL)] for r in rs]
            accs = [[None] * _NL for _ in range(_HPI)]
            ls = [[[None] * _NL for _ in range(_HPI)] for _ in range(2)]
            P = [dict() for _ in range(_NL)]
            pos = [0] * _NL
            for i, u in enumerate(_PRE):
                for j in range(_NL):
                    ls[1][u][j] = lp_scr[(hh * npre + i) * _NL + j]

            def add_l(w, u, j, p):
                n = p.shape[0] // 8
                ps = p.reshape(n, 8, 128).sum(axis=0) if n > 1 else p
                ls[w][u][j] = ps if ls[w][u][j] is None else ls[w][u][j] + ps

            def qk_seg(j, end):
                st = streams[j]
                end = min(end, len(st))
                if pos[j] >= end:
                    return False
                u = st[pos[j]][0]
                e = pos[j]
                while e < end and st[e][0] == u:
                    e += 1
                items = st[pos[j]:e]
                kk = jnp.concatenate(
                    [ksv[u][j][pl.ds(gof(j, n) * _GS, _GS), :] for (_, n) in items],
                    axis=0)
                p = jnp.exp2(jnp.dot(kk, qts[u][j], preferred_element_type=f32))
                add_l(0, u, j, p)
                for i, it in enumerate(items):
                    P[j][it] = p[i * _GS:(i + 1) * _GS]
                pos[j] = e
                return True

            def vpu(u, j, ns):
                nr = len(ns) * _GS
                r0 = kbrow[gof(j, ns[-1])]
                assert all(kbrow[gof(j, n)] == r0 + (ns[-1] - n) * _GS for n in ns)
                sv = None
                for d in range(DH):
                    qb = jnp.concatenate([qb_scr[j, rs[u] + d]] * len(ns), axis=0)
                    tt = kbv[u][j][pl.ds(r0, nr), pl.ds(d * 128, 128)] * qb
                    sv = tt if sv is None else sv + tt
                p = jnp.exp2(sv)
                add_l(1, u, j, p)
                for n in ns:
                    i = ns[-1] - n
                    P[j][(u, n)] = p[i * _GS:(i + 1) * _GS]

            def pre_pv(i):
                r = pl.multiple_of((hh * npre + i) * DH, DH)
                for j in range(_NL):
                    vc = vt_scr[j, :, pl.ds((nck - 1 - _CPRE) * _CK, _CK)]
                    ot2_scr[pl.ds(r, DH), pl.ds(j * 128, 128)] = jnp.dot(
                        vc, p_scr[(hh * npre + i) * _NL + j], preferred_element_type=f32)

            for i in range(len(_HEADPV)):
                for j in range(_NL):
                    qk_seg(j, _HEADPV[i])
                pre_pv(i)
            for m, (u, c) in enumerate(tiles):
                end = lastidx[(u, c)] + 1 + _DELTA
                more, first = True, True
                while more:
                    more = False
                    for j in range(_NL):
                        more |= qk_seg(j, end)
                        if first:
                            vpu(u, j, [c * _GPC + t for t in _vpu_run(u, c, j)])
                    first = False
                if m == len(tiles) - 1:
                    for i in range(len(_HEADPV), npre):
                        pre_pv(i)
                for j in range(_NL):
                    vc = vt_scr[j, :, pl.ds((nck - 1 - c) * _CK, _CK)]
                    tile = jnp.concatenate(
                        [P[j].pop((u, n))
                         for n in reversed(range(c * _GPC, (c + 1) * _GPC))], axis=0)
                    pv = jnp.dot(vc, tile, preferred_element_type=f32)
                    accs[u][j] = pv if accs[u][j] is None else pv + accs[u][j]
                    if c == nck - 1:
                        ot_scr[pl.ds(rs[u], DH), pl.ds(j * 128, 128)] = accs[u][j]
                        l_scr[j, pl.ds(pl.multiple_of((hh * _HPI + u) * 8, 8), 8), :] = (
                            ls[0][u][j] + ls[1][u][j])
            return carry

        lax.fori_loop(0, _H // _HPI, heads, 0)

    @pl.when(jnp.logical_not(safe))
    def _():
        ot2_scr[...] = jnp.zeros(ot2_scr.shape, f32)

        def head(h, carry):
            r = pl.multiple_of(h * DH, DH)
            qth = jnp.concatenate(
                [qt_scr[lt0 + j, pl.ds(r, DH), :] for j in range(_NL)], axis=1)

            def pass1(c, m):
                c0 = pl.multiple_of(c * _CK, _CK)
                s = jnp.dot(k_scr[pl.ds(c0, _CK), :], qth, preferred_element_type=f32)
                s_scr[pl.ds(c0, _CK), :] = s
                return jnp.maximum(m, s.reshape(_CK // 8, 8, _TQ).max(axis=0))

            m8 = lax.fori_loop(0, nck, pass1, jnp.full((8, _TQ), -jnp.inf, f32))
            m = jnp.max(m8, axis=0, keepdims=True)

            def pass2(c, carry2):
                l8, acc = carry2
                c0 = pl.multiple_of(c * _CK, _CK)
                p = jnp.exp2(s_scr[pl.ds(c0, _CK), :] - m)
                l8 = l8 + p.reshape(_CK // 8, 8, _TQ).sum(axis=0)
                acc = acc + jnp.dot(vt_scr[0, :, pl.ds(c0, _CK)], p,
                                    preferred_element_type=f32)
                return l8, acc

            l8, acc = lax.fori_loop(
                0, nck, pass2,
                (jnp.zeros((8, _TQ), f32), jnp.zeros((DH, _TQ), f32)))
            ot_scr[pl.ds(r, DH), :] = acc
            for j in range(_NL):
                l_scr[j, pl.ds(pl.multiple_of(h * 8, 8), 8), :] = (
                    l8[:, j * 128:(j + 1) * 128])
            return carry

        lax.fori_loop(0, _H, head, 0)

    @pl.when(step == 0)
    def _():
        for c in w_copies[3:]:
            c.wait()

    q0 = pl.multiple_of(step * _TQ, _TQ)
    ltn = jnp.minimum(step + 1, pl.num_programs(0) - 1) * _NL
    n1 = F // 128
    slots = _dense_slots([_PACE1] * n1 + list(_PACES), len(pre_heads) * _NL)
    lpart = {}

    def sign_bits(v):
        return lax.shift_right_logical(pltpu.bitcast(v, u32), jnp.uint32(31))

    def piece(unit, gi, n):
        i, j = divmod(unit, _NL)
        nr = n * _GS
        kbu = kb_scr.at[pl.ds(pl.multiple_of(z_scr[unit % _NZ], 8), kb_scr.shape[0])]
        r0 = kbrow[pre_g0[j] + gi]
        svs = [None, None]
        if gi == 0:
            build_qb(ltn, pre_heads[i], j)
        for d in range(DH):
            qb = jnp.concatenate([qb_scr[j, pre_heads[i] * DH + d]] * n, axis=0)
            tt = kbu[pl.ds(r0, nr), pl.ds(d * 128, 128)] * qb
            svs[d % 2] = tt if svs[d % 2] is None else svs[d % 2] + tt
        p = jnp.exp2(svs[0] + svs[1])
        p_scr[unit, pl.ds(gi * _GS, nr), :] = p
        ps = p.reshape(n, 8, 128).sum(axis=0) if n > 1 else p
        lpart[unit] = ps if gi == 0 else lpart[unit] + ps
        if gi + n == _GPC:
            lp_scr[unit] = lpart.pop(unit)
        return sign_bits(ps)

    lsum = []
    for j in range(_NL):
        lj = l_scr[j, pl.ds(0, _H, stride=8), :]
        for sub in range(1, 8):
            lj = lj + l_scr[j, pl.ds(sub, _H, stride=8), :]
        lsum.append(lj)
    rl = 1.0 / jnp.concatenate(lsum, axis=1)
    ots = []
    for hd in range(_H):
        t = ot_scr[pl.ds(hd * DH, DH), :]
        if hd in pre_heads:
            t = t + ot2_scr[pl.ds(pre_heads.index(hd) * DH, DH), :]
        ots.append(t * rl[hd:hd + 1])
    o = jnp.concatenate(ots, axis=0).T.astype(bf16)
    extra = {}
    for bi in range(16):
        rb, cb = divmod(bi, 4)
        extra[(_ODOT, 2 * bi)] = sign_bits(rl[rb * 8:rb * 8 + 8, cb * 128:(cb + 1) * 128])

    def gated(dot, ref, row0, c0, nc):
        gates = sorted({rg for (dd, rg) in list(slots) + list(extra) if dd == dot})
        rows = []
        r = 0
        for rg in gates + [_TQ // 16]:
            if rg > r:
                rows.append(ref[pl.ds(row0 + r * 8, (rg - r) * 8), pl.ds(c0, nc)])
            if rg < _TQ // 16:
                a = ref[pl.ds(row0 + rg * 8, 8), pl.ds(c0, 128)]
                if (dot, rg) in slots:
                    a = a | piece(*slots[(dot, rg)])
                if (dot, rg) in extra:
                    a = a | extra[(dot, rg)]
                b = ref[pl.ds(row0 + rg * 8, 8), pl.ds(c0 + 128, nc - 128)]
                rows.append(jnp.concatenate([a, b], axis=1))
                r = rg + 1
        lhs = jnp.concatenate(rows, axis=0) if len(rows) > 1 else rows[0]
        return pltpu.bitcast(lhs, bf16)

    q0h = pl.multiple_of(step * (_TQ // 2), _TQ // 2)
    dot = 0
    for n in range(n1):
        h = jnp.dot(gated(dot, xn_scr, q0h, 0, D), w1_scr[:, pl.ds(n * 128, 128)],
                    preferred_element_type=f32)
        h = h * (0.5 * jnp.tanh(0.5 * h) + 0.5)
        h_scr[:, pl.ds(n * 128, 128)] = pltpu.bitcast(h.astype(bf16), u32)
        dot += 1
    kfull = F // 512
    for nn in range(D // 128):
        acc = x_scr[pl.ds(q0, _TQ), pl.ds(nn * 128, 128)].astype(f32)
        for kk in range(kfull):
            acc = jnp.dot(gated(dot, h_scr, 0, kk * 512, 512),
                          w2_scr[pl.ds(kk * 512, 512), pl.ds(nn * 128, 128)],
                          preferred_element_type=f32) + acc
            dot += 1
        acc_scr[:, pl.ds(nn * 128, 128)] = acc
    rest = [(hd, j) for hd in range(_H) if hd not in pre_heads for j in range(_NL)]

    def release(val, k):
        n = len(rest) // 4
        for i in range(n):
            rr = i * (_TQ // 8) // n
            build_qb(ltn, *rest[k * n + i], val[rr * 8:rr * 8 + 8, :128])

    outs = []
    for nn in range(2):
        h3 = gated(dot, h_scr, 0, kfull * 512, 256)
        dot += 1
        acc = jnp.dot(h3, w2_scr[pl.ds(kfull * 512, 256), pl.ds(nn * 256, 256)],
                      preferred_element_type=f32) + acc_scr[:, pl.ds(nn * 256, 256)]
        release(acc, nn)
        outs += [acc[:, :128], acc[:, 128:]]
    for nn in range(D // 128):
        acc = jnp.dot(o, wo_scr[:, pl.ds(nn * 128, 128)],
                      preferred_element_type=f32) + outs[nn]
        if nn in (1, 2):
            release(acc, nn + 1)
        o_ref[:, pl.ds(nn * 128, 128)] = acc.astype(o_ref.dtype)


@jax.jit
def pallas_parallel_sum__grouped_kv_mqa__dense_activation_silu__prompt_kernel(
    A_x: jax.Array,
    A_wq: jax.Array,
    A_wk: jax.Array,
    A_wv: jax.Array,
    A_wo: jax.Array,
    B_x: jax.Array,
    B_w1: jax.Array,
    B_w2: jax.Array,
):
    B, S, D = A_x.shape
    DH = A_wk.shape[1]
    F = B_w1.shape[1]
    assert (B, S, D, DH, F) == (1, 2048, _H * 16, 16, 1792)
    x = A_x.reshape(S, D)
    bf16 = jnp.bfloat16
    f32 = jnp.float32
    nv = len(_plan(S)[1]) * _GS
    npre = len(_PRE) * (_H // _HPI)

    hbm = pl.BlockSpec(memory_space=pl.ANY)
    out = pl.pallas_call(
        functools.partial(_kernel, S=S, D=D, DH=DH, F=F),
        grid=(S // _TQ,),
        in_specs=[hbm] * 7,
        out_specs=pl.BlockSpec((_TQ, D), lambda i: (i, 0)),
        out_shape=jax.ShapeDtypeStruct((S, D), A_x.dtype),
        scratch_shapes=[
            pltpu.VMEM((S, D), bf16),
            pltpu.VMEM((D, D), bf16),
            pltpu.VMEM((D, D), bf16),
            pltpu.VMEM((D, F), bf16),
            pltpu.VMEM((F, D), bf16),
            pltpu.SemaphoreType.DMA((S // _RB,)),
            pltpu.SemaphoreType.DMA((6,)),
            pltpu.VMEM((S // 2, D), jnp.uint32),
            pltpu.VMEM((D + 2 * DH, D), bf16),
            pltpu.VMEM((S // 128, D, 128), f32),
            pltpu.VMEM((DH, S), f32),
            pltpu.VMEM((S, DH), f32),
            pltpu.VMEM((nv, DH * 128), f32),
            pltpu.VMEM((_NL, DH, S), f32),
            pltpu.VMEM((D, _TQ), f32),
            pltpu.VMEM((npre * DH, _TQ), f32),
            pltpu.VMEM((_NL, _H * 8 + 8, 128), f32),
            pltpu.VMEM((npre * _NL, _CK, 128), f32),
            pltpu.VMEM((npre * _NL, 8, 128), f32),
            pltpu.VMEM((_TQ // 2, F), jnp.uint32),
            pltpu.VMEM((_TQ, D), f32),
            pltpu.VMEM((_NL, D, 8, 128), f32),
            pltpu.VMEM((S, _TQ), f32),
            pltpu.SMEM((1,), jnp.int32),
            pltpu.SMEM((_NZ,), jnp.int32),
        ],
        compiler_params=pltpu.CompilerParams(
            dimension_semantics=("arbitrary",),
            vmem_limit_bytes=100 * 1024 * 1024),
    )(x, A_wq, A_wk.T, A_wv.T, A_wo, B_w1, B_w2)
    return out.reshape(B, S, D)
```

```python
import functools

import jax
import jax.numpy as jnp
from jax import lax
import jax.experimental.pallas as pl
import jax.experimental.pallas.tpu as pltpu

_H = 32
_TQ = 512
_NL = _TQ // 128
_CK = 128
_GS = 8
_GPC = _CK // _GS
_HPI = 8
_DELTA = 16
_ROT = 4
_RB = 256
_NZ = 64
_LOG2E = 1.4426950408889634
_SAFE_LOG2 = 58.0
_V_LO = 2.0 ** -30
_V_HI = 2.0 ** 30
_QG = 4
_PRE = (1, 3, 5, 7)
_CPRE = 14
_HEADPV = (6, 12)
_PACE1 = 18.0
_PACES = (8, 10, 11, 8, 8.5, 13, 9, 8, 13, 8, 14, 13, 16)
_ODOT = 25
_QBN = (0, 32, 20, 8, 16, 8, 16, 28)

_NT = (((1,), (1,)), ((), ()))


def _vpu_run(u, c, j):
    a = 12 - _ROT * j
    big = (c + (j in (0, 3))) % 2 == 0 and not (u in _PRE and c == _CPRE + 1)
    return tuple(range(a, a + (3 if big else 2)))


def _plan(S):
    NG = S // _GS
    nck = S // _CK
    gof = lambda j, n: (NG - 1 - n - _ROT * j) % NG
    tiles = [(u, c) for u in range(_HPI) for c in range(nck)
             if not (u in _PRE and c == _CPRE)]
    vg = {gof(j, _CPRE * _GPC + t) for j in range(_NL) for t in range(_GPC)}
    streams = [[] for _ in range(_NL)]
    for (u, c) in tiles:
        for j in range(_NL):
            for t in range(_GPC):
                if t in _vpu_run(u, c, j):
                    vg.add(gof(j, c * _GPC + t))
                else:
                    streams[j].append((u, c * _GPC + t))
    assert len({len(s) for s in streams}) == 1
    lastidx = {}
    for j in range(_NL):
        for i, (u, n) in enumerate(streams[j]):
            key = (u, n // _GPC)
            lastidx[key] = max(lastidx.get(key, 0), i)
    return gof, sorted(vg), tiles, streams, lastidx


def _dense_slots(paces, nunits):
    slots = {}
    unit, gi = 0, 0
    t = 48.0
    while unit < nunits:
        pace = paces[int(t // 512)]
        rem = _GPC - gi
        n = min(2 if (pace > 12 or rem == 4) else 3, rem)
        t += n * pace
        while (int(t // 512), int(t % 512) // 16) in slots:
            t = (t // 16 + 1) * 16
        assert t < 512 * len(paces)
        slots[(int(t // 512), int(t % 512) // 16)] = (unit, gi, n)
        gi += n
        if gi == _GPC:
            unit, gi = unit + 1, 0
    return slots


def _kernel(x_hbm, wq_hbm, wkt_hbm, wvt_hbm, wo_hbm, w1_hbm, w2_hbm, o_ref,
            x_scr, wq_scr, wo_scr, w1_scr, w2_scr, xsem, wsem,
            xn_scr, wkv_scr, wt_scr, qt_scr, kt_scr, k_scr, kb_scr, vt_scr, ot_scr, ot2_scr,
            l_scr, p_scr, lp_scr, h_scr, acc_scr, qb_scr, s_scr, flag_scr, z_scr,
            *, S, D, DH, F):
    f32 = jnp.float32
    bf16 = jnp.bfloat16
    u32 = jnp.uint32
    step = pl.program_id(0)
    nck = S // _CK
    nrb = S // _RB
    gof, vgroups, tiles, streams, lastidx = _plan(S)
    kbrow = {g: i * _GS for i, g in enumerate(vgroups)}
    npre = len(_PRE)
    pre_heads = [it * _HPI + u for it in range(_H // _HPI) for u in _PRE]
    pre_g0 = [gof(j, _CPRE * _GPC + _GPC - 1) for j in range(_NL)]

    def x_copy(i):
        return pltpu.make_async_copy(
            x_hbm.at[pl.ds(i * _RB, _RB)], x_scr.at[pl.ds(i * _RB, _RB)], xsem.at[i])

    w_copies = [
        pltpu.make_async_copy(wq_hbm, wq_scr, wsem.at[0]),
        pltpu.make_async_copy(wkt_hbm, wkv_scr.at[pl.ds(0, DH)], wsem.at[1]),
        pltpu.make_async_copy(wvt_hbm, wkv_scr.at[pl.ds(DH, DH)], wsem.at[2]),
        pltpu.make_async_copy(wo_hbm, wo_scr, wsem.at[3]),
        pltpu.make_async_copy(w1_hbm, w1_scr, wsem.at[4]),
        pltpu.make_async_copy(w2_hbm, w2_scr, wsem.at[5]),
    ]

    def build_qb(lt, hd, j, after=None):
        qq = qt_scr[lt + j, pl.ds(hd * DH, DH), :]
        if after is not None:
            zvec = jnp.full((8, 128), z_scr[0], jnp.int32).astype(u32)
            z = pltpu.bitcast(after, u32) & zvec
            qq = pltpu.bitcast(
                pltpu.bitcast(qq, u32) | jnp.concatenate([z, z], axis=0), f32)
        for d in range(DH):
            qb_scr[j, hd * DH + d] = jnp.broadcast_to(qq[d:d + 1], (8, 128))

    @pl.when(step == 0)
    def _():
        x_copy(0).start()
        for c in w_copies[:3]:
            c.start()
        x_copy(1).start()
        x_copy(2).start()
        for i in range(_NZ):
            z_scr[i] = 0

        def layernorm(i):
            x = x_scr[pl.ds(i * _RB, _RB), :].astype(f32)
            mu = jnp.mean(x, axis=-1, keepdims=True)
            xc = x - mu
            var = jnp.mean(xc * xc, axis=-1, keepdims=True)
            xn_scr[pl.ds(i * _RB // 2, _RB // 2), :] = pltpu.bitcast(
                (xc * lax.rsqrt(var + 1e-5)).astype(bf16), u32)

        def project(i):
            xn = pltpu.bitcast(xn_scr[pl.ds(i * _RB // 2, _RB // 2), :], bf16)
            t = lax.dot_general(pltpu.bitcast(wt_scr[...], bf16), xn, _NT,
                                preferred_element_type=f32)
            for j in range(_RB // 128):
                qt_scr[i * (_RB // 128) + j] = t[:D, j * 128:(j + 1) * 128]
            kt_scr[:, pl.ds(i * _RB, _RB)] = t[D:D + DH] * (DH ** -0.5 * _LOG2E)
            vt_scr[0, :, pl.ds(i * _RB, _RB)] = t[D + DH:]
            units = range(sum(_QBN[:i]), sum(_QBN[:i + 1]))
            for k, un in enumerate(units):
                cj, rr = divmod(k * 2 * (D // 8) // len(units), D // 8)
                build_qb(0, un % _H, un // _H,
                         t[rr * 8:rr * 8 + 8, cj * 128:(cj + 1) * 128])

        def post(i, stats):
            qmax, kmax, vmax = stats
            kt = kt_scr[:, pl.ds(i * _RB, _RB)]
            vt = vt_scr[0, :, pl.ds(i * _RB, _RB)]
            ktp = jnp.concatenate([kt, jnp.zeros((128 - DH, _RB), f32)], axis=0)
            kp = ktp.T
            k_scr[pl.ds(i * _RB, _RB), :] = kp[:, :DH]
            g0 = i * _RB // _GS
            gs = [g for g in vgroups if g0 <= g < g0 + _RB // _GS]
            ksel = jnp.concatenate(
                [kp[(g - g0) * _GS:(g - g0 + 1) * _GS] for g in gs], axis=0)
            nr = len(gs) * _GS
            lane = lax.broadcasted_iota(jnp.int32, (nr, 128), 1)
            for d in range(DH):
                col = jnp.sum(jnp.where(lane == d, ksel, 0.0), axis=1, keepdims=True)
                kb_scr[pl.ds(kbrow[gs[0]], nr), pl.ds(d * 128, 128)] = (
                    jnp.broadcast_to(col, (nr, 128)))
            q = jnp.concatenate(
                [qt_scr[i * (_RB // 128) + j] for j in range(_RB // 128)], axis=1)
            q2 = (q * q).reshape(_H // _QG, _QG, 2, 8, _RB)
            q2 = jnp.max(q2[:, :, 0] + q2[:, :, 1], axis=1)
            qmax = jnp.maximum(qmax, jnp.max(jnp.sum(q2, axis=1, keepdims=True), axis=0))
            kmax = jnp.maximum(kmax, jnp.sum(kt * kt, axis=0, keepdims=True))
            vmax = jnp.maximum(vmax, jnp.abs(vt))
            return qmax, kmax, vmax

        def pre_tile0(lo, hi):
            for i in range(lo, hi):
                for j in range(_NL):
                    kk = k_scr[pl.ds(pre_g0[j] * _GS, _CK), :]
                    qq = qt_scr[j, pl.ds(pre_heads[i] * DH, DH), :]
                    p = jnp.exp2(jnp.dot(kk, qq, preferred_element_type=f32))
                    p_scr[i * _NL + j] = p
                    lp_scr[i * _NL + j] = p.reshape(_GPC, 8, 128).sum(axis=0)

        x_copy(0).wait()
        for i in range(3, nrb):
            x_copy(i).start()
        layernorm(0)
        for c in w_copies[:3]:
            c.wait()
        wt_scr[pl.ds(0, D // 4), :] = pltpu.bitcast(
            wq_scr[:, pl.ds(0, D // 2)].astype(f32).T.astype(bf16), u32)
        x_copy(1).wait()
        x_copy(2).wait()
        wt_scr[pl.ds(D // 4, D // 4), :] = pltpu.bitcast(
            wq_scr[:, pl.ds(D // 2, D // 2)].astype(f32).T.astype(bf16), u32)
        wt_scr[pl.ds(D // 2, DH), :] = pltpu.bitcast(wkv_scr[...], u32)
        stats = (jnp.zeros((1, _RB), f32), jnp.zeros((1, _RB), f32),
                 jnp.zeros((DH, _RB), f32))
        layernorm(1)
        project(0)
        layernorm(2)
        project(1)
        for i in range(2, nrb + 2):
            if i == 2:
                for ii in range(3, nrb):
                    x_copy(ii).wait()
                for c in w_copies[3:]:
                    c.start()
            if i + 1 < nrb:
                layernorm(i + 1)
            if i < nrb:
                project(i)
            if i == nrb + 1:
                pre_tile0(0, len(pre_heads) // 2)
            stats = post(i - 2, stats)
        pre_tile0(len(pre_heads) // 2, len(pre_heads))
        vt_all = vt_scr[0]
        for j in range(1, _NL):
            vt_scr[j] = pltpu.roll(vt_all, _ROT * _GS * j, 1)
        qmax, kmax, vmax = [jnp.max(jnp.max(a, axis=0, keepdims=True), axis=1,
                                    keepdims=True)[0, 0] for a in stats]
        safe = jnp.logical_and(
            qmax * kmax <= _SAFE_LOG2 * _SAFE_LOG2,
            jnp.logical_and(vmax >= _V_LO, vmax <= _V_HI))
        flag_scr[0] = safe.astype(jnp.int32)

    safe = flag_scr[0] == 1
    lt0 = step * _NL

    @pl.when(safe)
    def _():
        def heads(hh, carry):
            rs = [pl.multiple_of((hh * _HPI + u) * DH, DH) for u in range(_HPI)]
            zs = [[pl.multiple_of(z_scr[u * _NL + j], 8) for j in range(_NL)]
                  for u in range(_HPI)]
            kbv = [[kb_scr.at[pl.ds(z, kb_scr.shape[0])] for z in zu] for zu in zs]
            ksv = [[k_scr.at[pl.ds(z, k_scr.shape[0])] for z in zu] for zu in zs]
            qts = [[qt_scr[lt0 + j, pl.ds(r, DH), :] for j in range(_NL)] for r in rs]
            accs = [[None] * _NL for _ in range(_HPI)]
            ls = [[[None] * _NL for _ in range(_HPI)] for _ in range(2)]
            P = [dict() for _ in range(_NL)]
            pos = [0] * _NL
            for i, u in enumerate(_PRE):
                for j in range(_NL):
                    ls[1][u][j] = lp_scr[(hh * npre + i) * _NL + j]

            def add_l(w, u, j, p):
                n = p.shape[0] // 8
                ps = p.reshape(n, 8, 128).sum(axis=0) if n > 1 else p
                ls[w][u][j] = ps if ls[w][u][j] is None else ls[w][u][j] + ps

            def qk_seg(j, end):
                st = streams[j]
                end = min(end, len(st))
                if pos[j] >= end:
                    return False
                u = st[pos[j]][0]
                e = pos[j]
                while e < end and st[e][0] == u:
                    e += 1
                items = st[pos[j]:e]
                kk = jnp.concatenate(
                    [ksv[u][j][pl.ds(gof(j, n) * _GS, _GS), :] for (_, n) in items],
                    axis=0)
                p = jnp.exp2(jnp.dot(kk, qts[u][j], preferred_element_type=f32))
                add_l(0, u, j, p)
                for i, it in enumerate(items):
                    P[j][it] = p[i * _GS:(i + 1) * _GS]
                pos[j] = e
                return True

            def vpu(u, j, ns):
                nr = len(ns) * _GS
                r0 = kbrow[gof(j, ns[-1])]
                assert all(kbrow[gof(j, n)] == r0 + (ns[-1] - n) * _GS for n in ns)
                sv = None
                for d in range(DH):
                    qb = jnp.concatenate([qb_scr[j, rs[u] + d]] * len(ns), axis=0)
                    tt = kbv[u][j][pl.ds(r0, nr), pl.ds(d * 128, 128)] * qb
                    sv = tt if sv is None else sv + tt
                p = jnp.exp2(sv)
                add_l(1, u, j, p)
                for n in ns:
                    i = ns[-1] - n
                    P[j][(u, n)] = p[i * _GS:(i + 1) * _GS]

            def pre_pv(i):
                r = pl.multiple_of((hh * npre + i) * DH, DH)
                for j in range(_NL):
                    vc = vt_scr[j, :, pl.ds((nck - 1 - _CPRE) * _CK, _CK)]
                    ot2_scr[pl.ds(r, DH), pl.ds(j * 128, 128)] = jnp.dot(
                        vc, p_scr[(hh * npre + i) * _NL + j], preferred_element_type=f32)

            for i in range(len(_HEADPV)):
                for j in range(_NL):
                    qk_seg(j, _HEADPV[i])
                pre_pv(i)
            for m, (u, c) in enumerate(tiles):
                end = lastidx[(u, c)] + 1 + _DELTA
                more, first = True, True
                while more:
                    more = False
                    for j in range(_NL):
                        more |= qk_seg(j, end)
                        if first:
                            vpu(u, j, [c * _GPC + t for t in _vpu_run(u, c, j)])
                    first = False
                if m == len(tiles) - 1:
                    for i in range(len(_HEADPV), npre):
                        pre_pv(i)
                for j in range(_NL):
                    vc = vt_scr[j, :, pl.ds((nck - 1 - c) * _CK, _CK)]
                    tile = jnp.concatenate(
                        [P[j].pop((u, n))
                         for n in reversed(range(c * _GPC, (c + 1) * _GPC))], axis=0)
                    pv = jnp.dot(vc, tile, preferred_element_type=f32)
                    accs[u][j] = pv if accs[u][j] is None else pv + accs[u][j]
                    if c == nck - 1:
                        ot_scr[pl.ds(rs[u], DH), pl.ds(j * 128, 128)] = accs[u][j]
                        l_scr[j, pl.ds(pl.multiple_of((hh * _HPI + u) * 8, 8), 8), :] = (
                            ls[0][u][j] + ls[1][u][j])
            return carry

        lax.fori_loop(0, _H // _HPI, heads, 0)

    @pl.when(jnp.logical_not(safe))
    def _():
        ot2_scr[...] = jnp.zeros(ot2_scr.shape, f32)

        def head(h, carry):
            r = pl.multiple_of(h * DH, DH)
            qth = jnp.concatenate(
                [qt_scr[lt0 + j, pl.ds(r, DH), :] for j in range(_NL)], axis=1)

            def pass1(c, m):
                c0 = pl.multiple_of(c * _CK, _CK)
                s = jnp.dot(k_scr[pl.ds(c0, _CK), :], qth, preferred_element_type=f32)
                s_scr[pl.ds(c0, _CK), :] = s
                return jnp.maximum(m, s.reshape(_CK // 8, 8, _TQ).max(axis=0))

            m8 = lax.fori_loop(0, nck, pass1, jnp.full((8, _TQ), -jnp.inf, f32))
            m = jnp.max(m8, axis=0, keepdims=True)

            def pass2(c, carry2):
                l8, acc = carry2
                c0 = pl.multiple_of(c * _CK, _CK)
                p = jnp.exp2(s_scr[pl.ds(c0, _CK), :] - m)
                l8 = l8 + p.reshape(_CK // 8, 8, _TQ).sum(axis=0)
                acc = acc + jnp.dot(vt_scr[0, :, pl.ds(c0, _CK)], p,
                                    preferred_element_type=f32)
                return l8, acc

            l8, acc = lax.fori_loop(
                0, nck, pass2,
                (jnp.zeros((8, _TQ), f32), jnp.zeros((DH, _TQ), f32)))
            ot_scr[pl.ds(r, DH), :] = acc
            for j in range(_NL):
                l_scr[j, pl.ds(pl.multiple_of(h * 8, 8), 8), :] = (
                    l8[:, j * 128:(j + 1) * 128])
            return carry

        lax.fori_loop(0, _H, head, 0)

    @pl.when(step == 0)
    def _():
        for c in w_copies[3:]:
            c.wait()

    q0 = pl.multiple_of(step * _TQ, _TQ)
    ltn = jnp.minimum(step + 1, pl.num_programs(0) - 1) * _NL
    n1 = F // 128
    slots = _dense_slots([_PACE1] * n1 + list(_PACES), len(pre_heads) * _NL)
    lpart = {}

    def sign_bits(v):
        return lax.shift_right_logical(pltpu.bitcast(v, u32), jnp.uint32(31))

    def piece(unit, gi, n):
        i, j = divmod(unit, _NL)
        nr = n * _GS
        kbu = kb_scr.at[pl.ds(pl.multiple_of(z_scr[unit % _NZ], 8), kb_scr.shape[0])]
        r0 = kbrow[pre_g0[j] + gi]
        svs = [None, None]
        if gi == 0:
            build_qb(ltn, pre_heads[i], j)
        for d in range(DH):
            qb = jnp.concatenate([qb_scr[j, pre_heads[i] * DH + d]] * n, axis=0)
            tt = kbu[pl.ds(r0, nr), pl.ds(d * 128, 128)] * qb
            svs[d % 2] = tt if svs[d % 2] is None else svs[d % 2] + tt
        p = jnp.exp2(svs[0] + svs[1])
        p_scr[unit, pl.ds(gi * _GS, nr), :] = p
        ps = p.reshape(n, 8, 128).sum(axis=0) if n > 1 else p
        lpart[unit] = ps if gi == 0 else lpart[unit] + ps
        if gi + n == _GPC:
            lp_scr[unit] = lpart.pop(unit)
        return sign_bits(ps)

    lsum = []
    for j in range(_NL):
        lj = l_scr[j, pl.ds(0, _H, stride=8), :]
        for sub in range(1, 8):
            lj = lj + l_scr[j, pl.ds(sub, _H, stride=8), :]
        lsum.append(lj)
    rl = 1.0 / jnp.concatenate(lsum, axis=1)
    ots = []
    for hd in range(_H):
        t = ot_scr[pl.ds(hd * DH, DH), :]
        if hd in pre_heads:
            t = t + ot2_scr[pl.ds(pre_heads.index(hd) * DH, DH), :]
        ots.append(t * rl[hd:hd + 1])
    o = jnp.concatenate(ots, axis=0).T.astype(bf16)
    extra = {}
    for bi in range(16):
        rb, cb = divmod(bi, 4)
        extra[(_ODOT, 2 * bi)] = sign_bits(rl[rb * 8:rb * 8 + 8, cb * 128:(cb + 1) * 128])

    def gated(dot, ref, row0, c0, nc):
        gates = sorted({rg for (dd, rg) in list(slots) + list(extra) if dd == dot})
        rows = []
        r = 0
        for rg in gates + [_TQ // 16]:
            if rg > r:
                rows.append(ref[pl.ds(row0 + r * 8, (rg - r) * 8), pl.ds(c0, nc)])
            if rg < _TQ // 16:
                a = ref[pl.ds(row0 + rg * 8, 8), pl.ds(c0, 128)]
                if (dot, rg) in slots:
                    a = a | piece(*slots[(dot, rg)])
                if (dot, rg) in extra:
                    a = a | extra[(dot, rg)]
                b = ref[pl.ds(row0 + rg * 8, 8), pl.ds(c0 + 128, nc - 128)]
                rows.append(jnp.concatenate([a, b], axis=1))
                r = rg + 1
        lhs = jnp.concatenate(rows, axis=0) if len(rows) > 1 else rows[0]
        return pltpu.bitcast(lhs, bf16)

    q0h = pl.multiple_of(step * (_TQ // 2), _TQ // 2)
    dot = 0
    for n in range(n1):
        h = jnp.dot(gated(dot, xn_scr, q0h, 0, D), w1_scr[:, pl.ds(n * 128, 128)],
                    preferred_element_type=f32)
        h = h * (0.5 * jnp.tanh(0.5 * h) + 0.5)
        h_scr[:, pl.ds(n * 128, 128)] = pltpu.bitcast(h.astype(bf16), u32)
        dot += 1
    kfull = F // 512
    for nn in range(D // 128):
        acc = x_scr[pl.ds(q0, _TQ), pl.ds(nn * 128, 128)].astype(f32)
        for kk in range(kfull):
            acc = jnp.dot(gated(dot, h_scr, 0, kk * 512, 512),
                          w2_scr[pl.ds(kk * 512, 512), pl.ds(nn * 128, 128)],
                          preferred_element_type=f32) + acc
            dot += 1
        acc_scr[:, pl.ds(nn * 128, 128)] = acc
    rest = [(hd, j) for hd in range(_H) if hd not in pre_heads for j in range(_NL)]

    def release(val, k):
        n = len(rest) // 4
        for i in range(n):
            rr = i * (_TQ // 8) // n
            build_qb(ltn, *rest[k * n + i], val[rr * 8:rr * 8 + 8, :128])

    outs = []
    for nn in range(2):
        h3 = gated(dot, h_scr, 0, kfull * 512, 256)
        dot += 1
        acc = jnp.dot(h3, w2_scr[pl.ds(kfull * 512, 256), pl.ds(nn * 256, 256)],
                      preferred_element_type=f32) + acc_scr[:, pl.ds(nn * 256, 256)]
        release(acc, nn)
        outs += [acc[:, :128], acc[:, 128:]]
    for nn in range(D // 128):
        acc = jnp.dot(o, wo_scr[:, pl.ds(nn * 128, 128)],
                      preferred_element_type=f32) + outs[nn]
        if nn in (1, 2):
            release(acc, nn + 1)
        o_ref[:, pl.ds(nn * 128, 128)] = acc.astype(o_ref.dtype)


@jax.jit
def pallas_parallel_sum__grouped_kv_mqa__dense_activation_silu__prompt_kernel(
    A_x: jax.Array,
    A_wq: jax.Array,
    A_wk: jax.Array,
    A_wv: jax.Array,
    A_wo: jax.Array,
    B_x: jax.Array,
    B_w1: jax.Array,
    B_w2: jax.Array,
):
    B, S, D = A_x.shape
    DH = A_wk.shape[1]
    F = B_w1.shape[1]
    assert (B, S, D, DH, F) == (1, 2048, _H * 16, 16, 1792)
    x = A_x.reshape(S, D)
    bf16 = jnp.bfloat16
    f32 = jnp.float32
    nv = len(_plan(S)[1]) * _GS
    npre = len(_PRE) * (_H // _HPI)

    hbm = pl.BlockSpec(memory_space=pl.ANY)
    out = pl.pallas_call(
        functools.partial(_kernel, S=S, D=D, DH=DH, F=F),
        grid=(S // _TQ,),
        in_specs=[hbm] * 7,
        out_specs=pl.BlockSpec((_TQ, D), lambda i: (i, 0)),
        out_shape=jax.ShapeDtypeStruct((S, D), A_x.dtype),
        scratch_shapes=[
            pltpu.VMEM((S, D), bf16),
            pltpu.VMEM((D, D), bf16),
            pltpu.VMEM((D, D), bf16),
            pltpu.VMEM((D, F), bf16),
            pltpu.VMEM((F, D), bf16),
            pltpu.SemaphoreType.DMA((S // _RB,)),
            pltpu.SemaphoreType.DMA((6,)),
            pltpu.VMEM((S // 2, D), jnp.uint32),
            pltpu.VMEM((2 * DH, D), bf16),
            pltpu.VMEM((D // 2 + DH, D), jnp.uint32),
            pltpu.VMEM((S // 128, D, 128), f32),
            pltpu.VMEM((DH, S), f32),
            pltpu.VMEM((S, DH), f32),
            pltpu.VMEM((nv, DH * 128), f32),
            pltpu.VMEM((_NL, DH, S), f32),
            pltpu.VMEM((D, _TQ), f32),
            pltpu.VMEM((npre * DH, _TQ), f32),
            pltpu.VMEM((_NL, _H * 8 + 8, 128), f32),
            pltpu.VMEM((npre * _NL, _CK, 128), f32),
            pltpu.VMEM((npre * _NL, 8, 128), f32),
            pltpu.VMEM((_TQ // 2, F), jnp.uint32),
            pltpu.VMEM((_TQ, D), f32),
            pltpu.VMEM((_NL, D, 8, 128), f32),
            pltpu.VMEM((S, _TQ), f32),
            pltpu.SMEM((1,), jnp.int32),
            pltpu.SMEM((_NZ,), jnp.int32),
        ],
        compiler_params=pltpu.CompilerParams(
            dimension_semantics=("arbitrary",),
            vmem_limit_bytes=100 * 1024 * 1024),
    )(x, A_wq, A_wk.T, A_wv.T, A_wo, B_w1, B_w2)
    return out.reshape(B, S, D)
```

```python
import functools

import jax
import jax.numpy as jnp
from jax import lax
import jax.experimental.pallas as pl
import jax.experimental.pallas.tpu as pltpu

_H = 32
_TQ = 512
_NL = _TQ // 128
_CK = 128
_GS = 8
_GPC = _CK // _GS
_HPI = 8
_DELTA = 16
_ROT = 4
_RB = 256
_NZ = 80
_LOG2E = 1.4426950408889634
_SAFE_LOG2 = 58.0
_V_LO = 2.0 ** -30
_V_HI = 2.0 ** 30
_QG = 4
_PRE = (0, 2, 4, 6, 7)
_CPRE = 14
_HEADPV = (6, 12)
_OPOS = 1
_PACE1 = 20.0
_PACES = (7.6,) * 3 + (None,) * 4 + (7.6,) * 11
_PACESA = (9.0,) * 14
_NVA = 17
_ODOT = 15
_EDOT = 23
_KT = ((0, 5, 8, 11), (1, 6, 9, 12), (2, 7, 10, 13), (3, 4))
_RELB = (17, 18, 19, 20)
_RELA = (22, 23, 24, 25, 26)

_NT = (((1,), (1,)), ((), ()))
_dot = functools.partial(jnp.dot, precision=lax.Precision.DEFAULT)


def _vpu_run(u, c, j):
    a = 12 - _ROT * j
    big = (c + (j in (0, 3))) % 2 == 0 and not (u in _PRE and c == _CPRE + 1)
    return tuple(range(a, a + (3 if big else 2)))


def _plan(S):
    NG = S // _GS
    nck = S // _CK
    gof = lambda j, n: (NG - 1 - n - _ROT * j) % NG
    tiles = [(u, c) for u in range(_HPI) for c in range(nck)
             if not (u in _PRE and c == _CPRE)]
    vg = set()
    streams = [[] for _ in range(_NL)]
    for (u, c) in tiles:
        for j in range(_NL):
            for t in range(_GPC):
                if t in _vpu_run(u, c, j):
                    vg.add(gof(j, c * _GPC + t))
                else:
                    streams[j].append((u, c * _GPC + t))
    assert len({len(s) for s in streams}) == 1
    lastidx = {}
    for j in range(_NL):
        for i, (u, n) in enumerate(streams[j]):
            key = (u, n // _GPC)
            lastidx[key] = max(lastidx.get(key, 0), i)
    return gof, sorted(vg), tiles, streams, lastidx


def _dense_slots(paces, nunits):
    slots = {}
    unit, gi = 0, 0
    t = 48.0
    while unit < nunits:
        pace = paces[int(t // 512)]
        if pace is None:
            t = (t // 512 + 1) * 512
            continue
        rem = _GPC - gi
        n = min(2 if (pace > 12 or rem == 4) else 3, rem)
        t += n * pace
        while ((int(t // 512), int(t % 512) // 16) in slots
               or (t < 512 * len(paces) and paces[int(t // 512)] is None)):
            t = (t // 16 + 1) * 16
        assert t < 512 * len(paces)
        slots[(int(t // 512), int(t % 512) // 16)] = (unit, gi, n)
        gi += n
        if gi == _GPC:
            unit, gi = unit + 1, 0
    return slots


def _kernel(x_hbm, wq_hbm, wkt_hbm, wvt_hbm, wo_hbm, w1_hbm, w2_hbm, o_ref,
            x_scr, wq_scr, wo_scr, w1_scr, w2_scr, xsem, wsem,
            xn_scr, wkv_scr, wt_scr, qt_scr, kt_scr, k_scr, kb_scr, kbp_scr, vt_scr,
            ot_scr, ot2_scr, l_scr, p_scr, lp_scr, h_scr, acc_scr, res_scr, qb_scr, s_scr, flag_scr, z_scr,
            *, S, D, DH, F):
    f32 = jnp.float32
    bf16 = jnp.bfloat16
    u32 = jnp.uint32
    step = pl.program_id(0)
    nck = S // _CK
    nrb = S // _RB
    gof, vgroups, tiles, streams, lastidx = _plan(S)
    kbrow = {g: i * _GS for i, g in enumerate(vgroups)}
    npre = len(_PRE)
    pre_heads = [it * _HPI + u for it in range(_H // _HPI) for u in _PRE]
    pre_g0 = [gof(j, _CPRE * _GPC + _GPC - 1) for j in range(_NL)]

    def x_copy(i):
        return pltpu.make_async_copy(
            x_hbm.at[pl.ds(i * _RB, _RB)], x_scr.at[pl.ds(i * _RB, _RB)], xsem.at[i])

    w_copies = [
        pltpu.make_async_copy(wq_hbm, wq_scr, wsem.at[0]),
        pltpu.make_async_copy(wkt_hbm, wkv_scr.at[pl.ds(0, DH)], wsem.at[1]),
        pltpu.make_async_copy(wvt_hbm, wkv_scr.at[pl.ds(DH, DH)], wsem.at[2]),
        pltpu.make_async_copy(wo_hbm, wo_scr, wsem.at[3]),
        pltpu.make_async_copy(w1_hbm, w1_scr, wsem.at[4]),
        pltpu.make_async_copy(w2_hbm, w2_scr, wsem.at[5]),
    ]

    def build_qb(lt, hd, j, after=None):
        qq = qt_scr[lt + j, pl.ds(hd * DH, DH), :]
        if after is not None:
            zvec = jnp.full((8, 128), z_scr[0], jnp.int32).astype(u32)
            z = pltpu.bitcast(after, u32) & zvec
            qq = pltpu.bitcast(
                pltpu.bitcast(qq, u32) | jnp.concatenate([z, z], axis=0), f32)
        for d in range(DH):
            qb_scr[j, hd * DH + d] = jnp.broadcast_to(qq[d:d + 1], (8, 128))

    n1 = F // 128

    def sign_bits(v):
        return lax.shift_right_logical(pltpu.bitcast(v, u32), jnp.uint32(31))

    def dense(tf, do_out, early=None):
        extra = {}
        if early is not None:
            extra[(_EDOT, 0)] = sign_bits(early)
        if do_out:
            lsum = []
            for j in range(_NL):
                lj = l_scr[j, pl.ds(0, _H, stride=8), :]
                for sub in range(1, 8):
                    lj = lj + l_scr[j, pl.ds(sub, _H, stride=8), :]
                lsum.append(lj)
            rl = 1.0 / jnp.concatenate(lsum, axis=1)
            ots = []
            for hd in range(_H):
                t = ot_scr[pl.ds(hd * DH, DH), :]
                if hd in pre_heads:
                    t = t + ot2_scr[pl.ds(pre_heads.index(hd) * DH, DH), :]
                ots.append(t * rl[hd:hd + 1])
            o = jnp.concatenate(ots, axis=0).T.astype(bf16)
            for bi in range(16):
                rb, cb = divmod(bi, 4)
                extra[(_ODOT, 2 * bi)] = sign_bits(
                    rl[rb * 8:rb * 8 + 8, cb * 128:(cb + 1) * 128])
        if tf is None:
            o_ref[...] = (_dot(o, wo_scr[...], preferred_element_type=f32)
                          + res_scr[...]).astype(o_ref.dtype)
            return
        ltn = tf * _NL
        q0 = tf * _TQ
        q0h = tf * (_TQ // 2)
        if not isinstance(tf, int):
            q0 = pl.multiple_of(q0, _TQ)
            q0h = pl.multiple_of(q0h, _TQ // 2)
        nvh = len(pre_heads) if do_out else _NVA
        slots = _dense_slots([_PACE1] * n1 + list(_PACES if do_out else _PACESA), nvh * _NL)
        lpart = {}
        kbus = {}

        def piece(unit, gi, n):
            i, j = divmod(unit, _NL)
            nr = n * _GS
            if unit not in kbus:
                kbus[unit] = kbp_scr.at[
                    pl.ds(pl.multiple_of(z_scr[unit % _NZ], 8), kbp_scr.shape[0])]
            kbu = kbus[unit]
            r0 = (pre_g0[j] - min(pre_g0) + gi) * _GS
            svs = [None, None]
            if gi == 0:
                build_qb(ltn, pre_heads[i], j)
            for d in range(DH):
                qb = jnp.concatenate([qb_scr[j, pre_heads[i] * DH + d]] * n, axis=0)
                tt = kbu[pl.ds(r0, nr), pl.ds(d * 128, 128)] * qb
                svs[d % 2] = tt if svs[d % 2] is None else svs[d % 2] + tt
            p = jnp.exp2(svs[0] + svs[1])
            p_scr[unit, pl.ds(gi * _GS, nr), :] = p
            ps = p.reshape(n, 8, 128).sum(axis=0) if n > 1 else p
            lpart[unit] = ps if gi == 0 else lpart[unit] + ps
            if gi + n == _GPC:
                lp_scr[unit] = lpart.pop(unit)
            return sign_bits(ps)

        def gated(dot, ref, row0, cts):
            gates = sorted({rg for (dd, rg) in list(slots) + list(extra) if dd == dot})
            rows = []
            r = 0
            for rg in gates + [_TQ // 16]:
                if rg > r:
                    rows.append(ref[pl.ds(row0 + r * 8, (rg - r) * 8),
                                    pl.ds(cts[0] * 128, 128)])
                if rg < _TQ // 16:
                    a = ref[pl.ds(row0 + rg * 8, 8), pl.ds(cts[0] * 128, 128)]
                    if (dot, rg) in slots:
                        a = a | piece(*slots[(dot, rg)])
                    if (dot, rg) in extra:
                        a = a | extra[(dot, rg)]
                    rows.append(a)
                    r = rg + 1
            cols = [jnp.concatenate(rows, axis=0) if len(rows) > 1 else rows[0]]
            cols += [ref[pl.ds(row0, _TQ // 2), pl.ds(ct * 128, 128)] for ct in cts[1:]]
            return pltpu.bitcast(jnp.concatenate(cols, axis=1), bf16)

        def wrows(cts, c0, nc):
            return jnp.concatenate(
                [w2_scr[pl.ds(ct * 128, 128), pl.ds(c0, nc)] for ct in cts], axis=0)

        rest = [(hd, j) for hd in range(_H) if hd not in pre_heads[:nvh]
                for j in range(_NL)]
        rel = list(_RELB if do_out else _RELA)

        def release(dot, val):
            if dot not in rel:
                return
            k = rel.index(dot)
            lo, hi = k * len(rest) // len(rel), (k + 1) * len(rest) // len(rel)
            for i in range(lo, hi):
                rr = (i - lo) * (_TQ // 8) // (hi - lo)
                build_qb(ltn, *rest[i], val[rr * 8:rr * 8 + 8, :128])

        dot = 0
        for n in range(n1):
            h = _dot(gated(dot, xn_scr, q0h, range(D // 128)),
                     w1_scr[:, pl.ds(n * 128, 128)], preferred_element_type=f32)
            h = h * (0.5 * jnp.tanh(0.5 * h) + 0.5)
            h_scr[:, pl.ds(n * 128, 128)] = pltpu.bitcast(h.astype(bf16), u32)
            dot += 1
        kfull = F // 512
        for nn in range(D // 128 + 1):
            if do_out and nn == _OPOS:
                for mm in range(D // 128):
                    acc = _dot(o, wo_scr[:, pl.ds(mm * 128, 128)], preferred_element_type=f32
                               ) + res_scr[:, pl.ds(mm * 128, 128)]
                    release(dot, acc)
                    dot += 1
                    o_ref[:, pl.ds(mm * 128, 128)] = acc.astype(o_ref.dtype)
            if nn == D // 128:
                break
            acc = x_scr[pl.ds(q0, _TQ), pl.ds(nn * 128, 128)].astype(f32)
            for kk in range(kfull):
                acc = _dot(gated(dot, h_scr, 0, _KT[kk]), wrows(_KT[kk], nn * 128, 128),
                           preferred_element_type=f32) + acc
                release(dot, acc)
                dot += 1
            acc_scr[:, pl.ds(nn * 128, 128)] = acc
        for nn in range(2):
            acc = _dot(gated(dot, h_scr, 0, _KT[kfull]), wrows(_KT[kfull], nn * 256, 256),
                       preferred_element_type=f32) + acc_scr[:, pl.ds(nn * 256, 256)]
            release(dot, acc)
            dot += 1
            res_scr[:, pl.ds(nn * 256, 256)] = acc

    @pl.when(step == 0)
    def _():
        x_copy(0).start()
        for c in w_copies[:3]:
            c.start()
        x_copy(1).start()
        x_copy(2).start()
        for i in range(_NZ):
            z_scr[i] = 0

        def layernorm(i):
            x = x_scr[pl.ds(i * _RB, _RB), :].astype(f32)
            mu = jnp.mean(x, axis=-1, keepdims=True)
            xc = x - mu
            var = jnp.mean(xc * xc, axis=-1, keepdims=True)
            xn_scr[pl.ds(i * _RB // 2, _RB // 2), :] = pltpu.bitcast(
                (xc * lax.rsqrt(var + 1e-5)).astype(bf16), u32)

        def project(i):
            xn = pltpu.bitcast(xn_scr[pl.ds(i * _RB // 2, _RB // 2), :], bf16)
            t = lax.dot_general(pltpu.bitcast(wt_scr[...], bf16), xn, _NT,
                                preferred_element_type=f32)
            for j in range(_RB // 128):
                qt_scr[i * (_RB // 128) + j] = t[:D, j * 128:(j + 1) * 128]
            kt_scr[:, pl.ds(i * _RB, _RB)] = t[D:D + DH] * (DH ** -0.5 * _LOG2E)
            vt_scr[0, :, pl.ds(i * _RB, _RB)] = t[D + DH:]

        def post(i, stats):
            qmax, kmax, vmax = stats
            kt = kt_scr[:, pl.ds(i * _RB, _RB)]
            vt = vt_scr[0, :, pl.ds(i * _RB, _RB)]
            ktp = jnp.concatenate([kt, jnp.zeros((128 - DH, _RB), f32)], axis=0)
            kp = ktp.T
            k_scr[pl.ds(i * _RB, _RB), :] = kp[:, :DH]
            g0 = i * _RB // _GS
            gs = [g for g in vgroups if g0 <= g < g0 + _RB // _GS]
            pg = list(range(min(pre_g0), max(pre_g0) + _GPC)) if i == 0 else []
            ga = sorted(set(gs + pg))
            ksel = jnp.concatenate(
                [kp[(g - g0) * _GS:(g - g0 + 1) * _GS] for g in ga], axis=0)
            nr = len(ga) * _GS
            lane = lax.broadcasted_iota(jnp.int32, (nr, 128), 1)
            for d in range(DH):
                col = jnp.sum(jnp.where(lane == d, ksel, 0.0), axis=1, keepdims=True)
                col = jnp.broadcast_to(col, (nr, 128))
                if pg:
                    k0 = ga.index(pg[0])
                    kbp_scr[:, pl.ds(d * 128, 128)] = col[k0 * _GS:(k0 + len(pg)) * _GS]
                    col = jnp.concatenate(
                        [col[ga.index(g) * _GS:(ga.index(g) + 1) * _GS] for g in gs], axis=0)
                kb_scr[pl.ds(kbrow[gs[0]], len(gs) * _GS), pl.ds(d * 128, 128)] = col
            q = jnp.concatenate(
                [qt_scr[i * (_RB // 128) + j] for j in range(_RB // 128)], axis=1)
            q2 = (q * q).reshape(_H // _QG, _QG, 2, 8, _RB)
            q2 = jnp.max(q2[:, :, 0] + q2[:, :, 1], axis=1)
            qmax = jnp.maximum(qmax, jnp.max(jnp.sum(q2, axis=1, keepdims=True), axis=0))
            kmax = jnp.maximum(kmax, jnp.sum(kt * kt, axis=0, keepdims=True))
            vmax = jnp.maximum(vmax, jnp.abs(vt))
            return qmax, kmax, vmax

        x_copy(0).wait()
        for i in range(3, nrb):
            x_copy(i).start()
        layernorm(0)
        for c in w_copies[:3]:
            c.wait()
        wt_scr[pl.ds(0, D // 4), :] = pltpu.bitcast(
            wq_scr[:, pl.ds(0, D // 2)].astype(f32).T.astype(bf16), u32)
        x_copy(1).wait()
        x_copy(2).wait()
        wt_scr[pl.ds(D // 4, D // 4), :] = pltpu.bitcast(
            wq_scr[:, pl.ds(D // 2, D // 2)].astype(f32).T.astype(bf16), u32)
        wt_scr[pl.ds(D // 2, DH), :] = pltpu.bitcast(wkv_scr[...], u32)
        stats = (jnp.zeros((1, _RB), f32), jnp.zeros((1, _RB), f32),
                 jnp.zeros((DH, _RB), f32))
        layernorm(1)
        project(0)
        layernorm(2)
        project(1)
        for i in range(2, nrb + 2):
            if i == 2:
                w_copies[4].start()
                w_copies[5].start()
                for ii in range(3, nrb):
                    x_copy(ii).wait()
            if i + 1 < nrb:
                layernorm(i + 1)
            if i < nrb:
                project(i)
            if i == nrb - 1:
                for ii in range(_NVA, len(pre_heads)):
                    for j in range(_NL):
                        p = jnp.exp2(_dot(k_scr[pl.ds(pre_g0[j] * _GS, _CK), :],
                                          qt_scr[j, pl.ds(pre_heads[ii] * DH, DH), :],
                                          preferred_element_type=f32))
                        p_scr[ii * _NL + j] = p
                        lp_scr[ii * _NL + j] = p.reshape(_GPC, 8, 128).sum(axis=0)
            if i == nrb:
                w_copies[4].wait()
                w_copies[5].wait()
                w_copies[3].start()
            stats = post(i - 2, stats)
        vt_all = vt_scr[0]
        for j in range(1, _NL):
            vt_scr[j] = pltpu.roll(vt_all, _ROT * _GS * j, 1)
        qmax, kmax, vmax = [jnp.max(jnp.max(a, axis=0, keepdims=True), axis=1,
                                    keepdims=True)[0, 0] for a in stats]
        safe = jnp.logical_and(
            qmax * kmax <= _SAFE_LOG2 * _SAFE_LOG2,
            jnp.logical_and(vmax >= _V_LO, vmax <= _V_HI))
        flag_scr[0] = safe.astype(jnp.int32)
        tok = stats[0] + stats[1] + stats[2][:8] + stats[2][8:]
        dense(0, False, tok[:, :128] + tok[:, 128:])

    safe = flag_scr[0] == 1
    lt0 = step * _NL

    def fast_path():
        def heads(hh, carry):
            rs = [pl.multiple_of((hh * _HPI + u) * DH, DH) for u in range(_HPI)]
            zs = [[pl.multiple_of(z_scr[u * _NL + j], 8) for j in range(_NL)]
                  for u in range(_HPI)]
            kbv = [[kb_scr.at[pl.ds(z, kb_scr.shape[0])] for z in zu] for zu in zs]
            ksv = [[k_scr.at[pl.ds(z, k_scr.shape[0])] for z in zu] for zu in zs]
            qts = [[qt_scr[lt0 + j, pl.ds(r, DH), :] for j in range(_NL)] for r in rs]
            accs = [[None] * _NL for _ in range(_HPI)]
            ls = [[[None] * _NL for _ in range(_HPI)] for _ in range(2)]
            P = [dict() for _ in range(_NL)]
            pos = [0] * _NL
            qbs = {}
            for i, u in enumerate(_PRE):
                for j in range(_NL):
                    ls[1][u][j] = lp_scr[(hh * npre + i) * _NL + j]

            def add_l(w, u, j, p):
                n = p.shape[0] // 8
                ps = p.reshape(n, 8, 128).sum(axis=0) if n > 1 else p
                ls[w][u][j] = ps if ls[w][u][j] is None else ls[w][u][j] + ps

            def qk_seg(j, end):
                st = streams[j]
                end = min(end, len(st))
                if pos[j] >= end:
                    return False
                u = st[pos[j]][0]
                e = pos[j]
                while e < end and st[e][0] == u:
                    e += 1
                items = st[pos[j]:e]
                kk = jnp.concatenate(
                    [ksv[u][j][pl.ds(gof(j, n) * _GS, _GS), :] for (_, n) in items],
                    axis=0)
                p = jnp.exp2(_dot(kk, qts[u][j], preferred_element_type=f32))
                add_l(0, u, j, p)
                for i, it in enumerate(items):
                    P[j][it] = p[i * _GS:(i + 1) * _GS]
                pos[j] = e
                return True

            def vpu(u, j, ns):
                nr = len(ns) * _GS
                r0 = kbrow[gof(j, ns[-1])]
                assert all(kbrow[gof(j, n)] == r0 + (ns[-1] - n) * _GS for n in ns)
                sv = None
                for d in range(DH):
                    if (u, j, d) not in qbs:
                        qbs[(u, j, d)] = qb_scr[j, rs[u] + d]
                    if (u, j, d, nr) not in qbs:
                        qbs[(u, j, d, nr)] = jnp.concatenate(
                            [qbs[(u, j, d)]] * len(ns), axis=0)
                    qb = qbs[(u, j, d, nr)]
                    tt = kbv[u][j][pl.ds(r0, nr), pl.ds(d * 128, 128)] * qb
                    sv = tt if sv is None else sv + tt
                p = jnp.exp2(sv)
                add_l(1, u, j, p)
                for n in ns:
                    i = ns[-1] - n
                    P[j][(u, n)] = p[i * _GS:(i + 1) * _GS]

            def pre_pv(i):
                r = pl.multiple_of((hh * npre + i) * DH, DH)
                for j in range(_NL):
                    vc = vt_scr[j, :, pl.ds((nck - 1 - _CPRE) * _CK, _CK)]
                    ot2_scr[pl.ds(r, DH), pl.ds(j * 128, 128)] = _dot(
                        vc, p_scr[(hh * npre + i) * _NL + j], preferred_element_type=f32)

            for i in range(len(_HEADPV)):
                for j in range(_NL):
                    qk_seg(j, _HEADPV[i])
                pre_pv(i)
            for m, (u, c) in enumerate(tiles):
                end = lastidx[(u, c)] + 1 + _DELTA
                more, first = True, True
                while more:
                    more = False
                    for j in range(_NL):
                        more |= qk_seg(j, end)
                        if first:
                            vpu(u, j, [c * _GPC + t for t in _vpu_run(u, c, j)])
                    first = False
                if m == len(tiles) - 1:
                    for i in range(len(_HEADPV), npre):
                        pre_pv(i)
                for j in range(_NL):
                    vc = vt_scr[j, :, pl.ds((nck - 1 - c) * _CK, _CK)]
                    tile = jnp.concatenate(
                        [P[j].pop((u, n))
                         for n in reversed(range(c * _GPC, (c + 1) * _GPC))], axis=0)
                    pv = _dot(vc, tile, preferred_element_type=f32)
                    accs[u][j] = pv if accs[u][j] is None else pv + accs[u][j]
                    if c == nck - 1:
                        ot_scr[pl.ds(rs[u], DH), pl.ds(j * 128, 128)] = accs[u][j]
                        l_scr[j, pl.ds(pl.multiple_of((hh * _HPI + u) * 8, 8), 8), :] = (
                            ls[0][u][j] + ls[1][u][j])
            return carry

        lax.fori_loop(0, _H // _HPI, heads, 0)

    def general_path():
        ot2_scr[...] = jnp.zeros(ot2_scr.shape, f32)

        def head(h, carry):
            r = pl.multiple_of(h * DH, DH)
            qth = jnp.concatenate(
                [qt_scr[lt0 + j, pl.ds(r, DH), :] for j in range(_NL)], axis=1)

            def pass1(c, m):
                c0 = pl.multiple_of(c * _CK, _CK)
                s = _dot(k_scr[pl.ds(c0, _CK), :], qth, preferred_element_type=f32)
                s_scr[pl.ds(c0, _CK), :] = s
                return jnp.maximum(m, s.reshape(_CK // 8, 8, _TQ).max(axis=0))

            m8 = lax.fori_loop(0, nck, pass1, jnp.full((8, _TQ), -jnp.inf, f32))
            m = jnp.max(m8, axis=0, keepdims=True)

            def pass2(c, carry2):
                l8, acc = carry2
                c0 = pl.multiple_of(c * _CK, _CK)
                p = jnp.exp2(s_scr[pl.ds(c0, _CK), :] - m)
                l8 = l8 + p.reshape(_CK // 8, 8, _TQ).sum(axis=0)
                acc = acc + _dot(vt_scr[0, :, pl.ds(c0, _CK)], p,
                                    preferred_element_type=f32)
                return l8, acc

            l8, acc = lax.fori_loop(
                0, nck, pass2,
                (jnp.zeros((8, _TQ), f32), jnp.zeros((DH, _TQ), f32)))
            ot_scr[pl.ds(r, DH), :] = acc
            for j in range(_NL):
                l_scr[j, pl.ds(pl.multiple_of(h * 8, 8), 8), :] = (
                    l8[:, j * 128:(j + 1) * 128])
            return carry

        lax.fori_loop(0, _H, head, 0)

    lax.cond(safe, fast_path, general_path)

    @pl.when(step == 0)
    def _():
        w_copies[3].wait()

    lax.cond(step < pl.num_programs(0) - 1,
             lambda: dense(step + 1, True), lambda: dense(None, True))


@jax.jit
def pallas_parallel_sum__grouped_kv_mqa__dense_activation_silu__prompt_kernel(
    A_x: jax.Array,
    A_wq: jax.Array,
    A_wk: jax.Array,
    A_wv: jax.Array,
    A_wo: jax.Array,
    B_x: jax.Array,
    B_w1: jax.Array,
    B_w2: jax.Array,
):
    B, S, D = A_x.shape
    DH = A_wk.shape[1]
    F = B_w1.shape[1]
    assert (B, S, D, DH, F) == (1, 2048, _H * 16, 16, 1792)
    x = A_x.reshape(S, D)
    bf16 = jnp.bfloat16
    f32 = jnp.float32
    nv = len(_plan(S)[1]) * _GS
    npre = len(_PRE) * (_H // _HPI)

    hbm = pl.BlockSpec(memory_space=pl.ANY)
    out = pl.pallas_call(
        functools.partial(_kernel, S=S, D=D, DH=DH, F=F),
        grid=(S // _TQ,),
        in_specs=[hbm] * 7,
        out_specs=pl.BlockSpec((_TQ, D), lambda i: (i, 0)),
        out_shape=jax.ShapeDtypeStruct((S, D), A_x.dtype),
        scratch_shapes=[
            pltpu.VMEM((S, D), bf16),
            pltpu.VMEM((D, D), bf16),
            pltpu.VMEM((D, D), bf16),
            pltpu.VMEM((D, F), bf16),
            pltpu.VMEM((F, D), bf16),
            pltpu.SemaphoreType.DMA((S // _RB,)),
            pltpu.SemaphoreType.DMA((6,)),
            pltpu.VMEM((S // 2, D), jnp.uint32),
            pltpu.VMEM((2 * DH, D), bf16),
            pltpu.VMEM((D // 2 + DH, D), jnp.uint32),
            pltpu.VMEM((S // 128, D, 128), f32),
            pltpu.VMEM((DH, S), f32),
            pltpu.VMEM((S, DH), f32),
            pltpu.VMEM((nv, DH * 128), f32),
            pltpu.VMEM(((_GPC + _ROT * (_NL - 1)) * _GS, DH * 128), f32),
            pltpu.VMEM((_NL, DH, S), f32),
            pltpu.VMEM((D, _TQ), f32),
            pltpu.VMEM((npre * DH, _TQ), f32),
            pltpu.VMEM((_NL, _H * 8 + 8, 128), f32),
            pltpu.VMEM((npre * _NL, _CK, 128), f32),
            pltpu.VMEM((npre * _NL, 8, 128), f32),
            pltpu.VMEM((_TQ // 2, F), jnp.uint32),
            pltpu.VMEM((_TQ, D), f32),
            pltpu.VMEM((_TQ, D), f32),
            pltpu.VMEM((_NL, D, 8, 128), f32),
            pltpu.VMEM((S, _TQ), f32),
            pltpu.SMEM((1,), jnp.int32),
            pltpu.SMEM((_NZ,), jnp.int32),
        ],
        compiler_params=pltpu.CompilerParams(
            dimension_semantics=("arbitrary",),
            vmem_limit_bytes=100 * 1024 * 1024),
    )(x, A_wq, A_wk.T, A_wv.T, A_wo, B_w1, B_w2)
    return out.reshape(B, S, D)
```
